```python
import jax
import jax.numpy as jnp

def _softmax(x, axis=-1):
    return jax.nn.softmax(x, axis=axis)
def _gelu(x):
    return jax.nn.gelu(x, approximate=True)
def _silu(x):
    return jax.nn.silu(x)
def _sigmoid(x):
    return jax.nn.sigmoid(x)
def _layernorm(x, axis=-1, eps=1e-5):
    m = jnp.mean(x, axis=axis, keepdims=True)
    v = jnp.var(x, axis=axis, keepdims=True)
    return (x - m) / jnp.sqrt(v + eps)
def _scatter_add(tgt, idx, src, axis=0):
    return tgt.at[idx].add(src)
def _segment_sum(src, seg, n):
    return jax.ops.segment_sum(src, seg, n)
class _Rng:
    def __init__(self, key):
        self._k = key
    def _next(self):
        self._k, sub = jax.random.split(self._k)
        return sub
    def normal(self, shape):
        return jax.random.normal(self._next(), shape, dtype=jnp.bfloat16)
    def randint(self, lo, hi, shape):
        return jax.random.randint(self._next(), shape, lo, hi, dtype=jnp.int32)
    def uniform(self, shape, lo=0.0, hi=1.0):
        return jax.random.uniform(self._next(), shape, jnp.bfloat16, lo, hi)
    def permutation(self, n):
        return jax.random.permutation(self._next(), n)


kernel_name = 'interleave_layers__sliding_local_dilated__dense_activation_gelu__prompt'

def setup_inputs():
    _rng = _Rng(jax.random.key(int.from_bytes(__import__("os").urandom(4), "little")))
    _w = (lambda a: (lambda t: t.astype(jnp.bfloat16) if jnp.issubdtype(t.dtype, jnp.floating) else t)(jnp.asarray(a)))
    def _A_setup():
        B, S, D = 1, 2048, 1024
        return {
            "x": _w((lambda *s: _rng.normal(s) * 0.05)(B, S, D)),
            "wqkv": _w((lambda *s: _rng.normal(s) * 0.05)(D, 3 * D)),
            "wo": _w((lambda *s: _rng.normal(s) * 0.05)(D, D)),
        }
    _A_in = _A_setup()

    def _B_setup():
        B, S, D, F = 1, 2048, 1024, 3584
        return {
            "x": _w((lambda *s: _rng.normal(s) * 0.05)(B, S, D)),
            "w1": _w((lambda *s: _rng.normal(s) * 0.05)(D, F) * (D ** -0.5)),
            "b1": _w((lambda *s: _rng.normal(s) * 0.05)(F) * 0.01),
            "w2": _w((lambda *s: _rng.normal(s) * 0.05)(F, D) * (F ** -0.5)),
            "b2": _w((lambda *s: _rng.normal(s) * 0.05)(D) * 0.01),
        }
    _B_in = _B_setup()

    return {
        "A_x": _A_in["x"],
        "A_wqkv": _A_in["wqkv"],
        "A_wo": _A_in["wo"],
        "B_x": _B_in["x"],
        "B_w1": _B_in["w1"],
        "B_b1": _B_in["b1"],
        "B_w2": _B_in["w2"],
        "B_b2": _B_in["b2"],
    }

def reference(A_x, A_wqkv, A_wo, B_x, B_w1, B_b1, B_w2, B_b2):
    def _A_ref(x, wqkv, wo):
        B, S, D = x.shape
        H = 32; Dh = D // H
        W, dil = 8, 2
        qkv = (lambda x, *d: x.transpose(*d))((x @ wqkv).reshape(B, S, 3, H, Dh), 2, 0, 3, 1, 4)
        q, k, v = qkv[0], qkv[1], qkv[2]
        scale = Dh ** -0.5
        pos = jnp.arange(S)
        off = jnp.arange(W) * dil
        idx = pos[:, None] - off[None, :]
        mask = idx >= 0
        idx_c = jnp.where(mask, idx, 0).reshape(-1)
        kg = k[:, :, idx_c, :].reshape(B, H, S, W, Dh)
        vg = v[:, :, idx_c, :].reshape(B, H, S, W, Dh)
        logits = jnp.einsum("bhsd,bhswd->bhsw", q, kg) * scale
        logits = jnp.where(mask[None, None, :, :], logits, -1e9)
        attn = _softmax(logits, axis=-1)
        o = jnp.einsum("bhsw,bhswd->bhsd", attn, vg)
        return (lambda x, *d: x.transpose(*d))(o, 0, 2, 1, 3).reshape(B, S, D) @ wo

    def _B_ref(x, w1, b1, w2, b2):
        h = jnp.einsum("bsd,df->bsf", x, w1) + b1
        h = _gelu(h)
        return jnp.einsum("bsf,fd->bsd", h, w2) + b2

    x = A_x
    x = x + _A_ref(_layernorm(x, axis=-1), A_wqkv, A_wo)
    x = x + _B_ref(_layernorm(x, axis=-1), B_w1, B_b1, B_w2, B_b2)
    x = x + _A_ref(_layernorm(x, axis=-1), A_wqkv, A_wo)
    x = x + _B_ref(_layernorm(x, axis=-1), B_w1, B_b1, B_w2, B_b2)
    return x
```

```python
import functools
import math

import jax
import jax.numpy as jnp
from jax import lax
import jax.experimental.pallas as pl
import jax.experimental.pallas.tpu as pltpu

H = 32
W = 8
DIL = 2
HALO = 16
LANES = 128
EPS = 1e-5
F32 = jnp.float32
BF16 = jnp.bfloat16


def _layernorm(x):
    m = jnp.mean(x, axis=-1, keepdims=True)
    xc = x - m
    v = jnp.mean(xc * xc, axis=-1, keepdims=True)
    return xc * lax.rsqrt(v + EPS)


def _gelu(x):
    c = math.sqrt(2.0 / math.pi)
    hx = 0.5 * x
    return hx + hx * jnp.tanh(x * (c + (c * 0.044715) * (x * x)))


def _butterfly(tiles, idx, axis, size, unit):
    tiles = list(tiles)
    for tb in (4, 2, 1):
        s = tb * unit
        m = (idx & s) == 0
        new = list(tiles)
        for g in range(8):
            if g & tb:
                continue
            x, y = tiles[g], tiles[g | tb]
            new[g] = jnp.where(m, x, pltpu.roll(y, s, axis))
            new[g | tb] = jnp.where(m, pltpu.roll(x, size - s, axis), y)
        tiles = new
    return tiles


def _permute_cols(w_ref, col0):
    rb = 32

    def body(r, carry):
        r0 = pl.multiple_of(r * rb, rb)
        tiles = [pltpu.bitcast(w_ref[pl.ds(r0, rb), pl.ds(col0 + LANES * g, LANES)], jnp.uint32)
                 for g in range(8)]
        lane = lax.broadcasted_iota(jnp.int32, tiles[0].shape, 1)
        tiles = _butterfly(tiles, lane, 1, LANES, 4)
        for g in range(8):
            w_ref[pl.ds(r0, rb), pl.ds(col0 + LANES * g, LANES)] = pltpu.bitcast(tiles[g], BF16)
        return carry

    lax.fori_loop(0, w_ref.shape[0] // rb, body, 0)


def _permute_rows(w_ref):
    def body(t, carry):
        a = t // 8
        n = t % 8
        r0 = pl.multiple_of(a * 32, 32)
        c0 = pl.multiple_of(n * LANES, LANES)
        tiles = [pltpu.bitcast(w_ref[pl.ds(r0 + LANES * g, 32), pl.ds(c0, LANES)], jnp.uint32)
                 for g in range(8)]
        row = lax.broadcasted_iota(jnp.int32, tiles[0].shape, 0)
        tiles = _butterfly(tiles, row, 0, 16, 2)
        for g in range(8):
            w_ref[pl.ds(r0 + LANES * g, 32), pl.ds(c0, LANES)] = pltpu.bitcast(tiles[g], BF16)
        return carry

    lax.fori_loop(0, 32, body, 0)


def _attn_rows(q_s, k_s, v_s, o_s, r0, R, pos0):
    lane = lax.broadcasted_iota(jnp.int32, (R, LANES), 1)
    m1 = (lane & 1) == 0
    m2 = (lane & 2) == 0
    q = [q_s[g, pl.ds(r0, R), :] for g in range(8)]
    logits = []
    for w in range(W):
        off = r0 + HALO - DIL * w
        acc = q[0] * k_s[0, pl.ds(off, R), :]
        for g in range(1, 8):
            acc = acc + q[g] * k_s[g, pl.ds(off, R), :]
        acc = acc + jnp.where(m1, pltpu.roll(acc, LANES - 1, 1), pltpu.roll(acc, 1, 1))
        acc = acc + jnp.where(m2, pltpu.roll(acc, LANES - 2, 1), pltpu.roll(acc, 2, 1))
        if pos0 is not None and w > 0:
            pos = pos0 + lax.broadcasted_iota(jnp.int32, (R, LANES), 0)
            acc = jnp.where(pos >= DIL * w, acc, -1e9)
        logits.append(acc)
    mx = logits[0]
    for w in range(1, W):
        mx = jnp.maximum(mx, logits[w])
    p = [jnp.exp2(l - mx) for l in logits]
    den = p[0]
    for w in range(1, W):
        den = den + p[w]
    inv = 1.0 / den
    p = [pw * inv for pw in p]
    for g in range(8):
        acc = p[0] * v_s[g, pl.ds(r0 + HALO, R), :]
        for w in range(1, W):
            acc = acc + p[w] * v_s[g, pl.ds(r0 + HALO - DIL * w, R), :]
        o_s[pl.ds(r0, R), pl.ds(LANES * g, LANES)] = acc.astype(BF16)


def _kernel(x_ref, wqkv_hbm, wo_hbm, w1_hbm, b1_ref, w2_hbm, b2_ref, out_ref,
            wqkv_s, wo_s, w1_s, w2_s, q_s, k_s, v_s, o_s, sems, *, T, R, FC):
    i = pl.program_id(0)
    D = x_ref.shape[1]
    F = w1_s.shape[1]
    qscale = (D // H) ** -0.5 * math.log2(math.e)

    def cp_qkv(p):
        return pltpu.make_async_copy(wqkv_hbm.at[:, pl.ds(p * D, D)], wqkv_s.at[:, pl.ds(p * D, D)], sems.at[p])

    cp_wo = pltpu.make_async_copy(wo_hbm, wo_s, sems.at[3])
    cp_w1 = pltpu.make_async_copy(w1_hbm, w1_s, sems.at[4])
    cp_w2 = pltpu.make_async_copy(w2_hbm, w2_s, sems.at[5])

    @pl.when(i == 0)
    def _():
        for p in range(3):
            cp_qkv(p).start()
        cp_wo.start()
        cp_w1.start()
        cp_w2.start()
        k_s[:, :, pl.ds(T, HALO), :] = jnp.zeros((2, 8, HALO, LANES), F32)
        v_s[:, :, pl.ds(T, HALO), :] = jnp.zeros((2, 8, HALO, LANES), F32)
        for p in range(3):
            cp_qkv(p).wait()
            _permute_cols(wqkv_s, p * D)
        cp_wo.wait()
        _permute_rows(wo_s)

    x = x_ref[...].astype(F32)
    for layer in range(2):
        kl = k_s.at[layer]
        vl = v_s.at[layer]
        kl[:, pl.ds(0, HALO), :] = kl[:, pl.ds(T, HALO), :]
        vl[:, pl.ds(0, HALO), :] = vl[:, pl.ds(T, HALO), :]
        xn = _layernorm(x).astype(BF16)
        q = jnp.dot(xn, wqkv_s[:, pl.ds(0, D)], preferred_element_type=F32) * qscale
        for g in range(8):
            q_s[g] = q[:, LANES * g:LANES * (g + 1)]
        k = jnp.dot(xn, wqkv_s[:, pl.ds(D, D)], preferred_element_type=F32)
        for g in range(8):
            kl[g, pl.ds(HALO, T), :] = k[:, LANES * g:LANES * (g + 1)]
        v = jnp.dot(xn, wqkv_s[:, pl.ds(2 * D, D)], preferred_element_type=F32)
        for g in range(8):
            vl[g, pl.ds(HALO, T), :] = v[:, LANES * g:LANES * (g + 1)]
        for c in range(T // R):
            _attn_rows(q_s, kl, vl, o_s, c * R, R, (i * T + c * R) if c * R < HALO else None)
        x = x + jnp.dot(o_s[...], wo_s[...], preferred_element_type=F32)

        if layer == 0:
            @pl.when(i == 0)
            def _():
                cp_w1.wait()
                cp_w2.wait()

        xn = _layernorm(x).astype(BF16)
        x = x + b2_ref[...].astype(F32)
        for c in range(F // FC):
            h = jnp.dot(xn, w1_s[:, pl.ds(c * FC, FC)], preferred_element_type=F32)
            h = _gelu(h + b1_ref[:, pl.ds(c * FC, FC)].astype(F32)).astype(BF16)
            x = x + jnp.dot(h, w2_s[pl.ds(c * FC, FC), :], preferred_element_type=F32)
    out_ref[...] = x.astype(out_ref.dtype)


def _forward(A_x, A_wqkv, A_wo, B_w1, B_b1, B_w2, B_b2, T=256, R=16, FC=512):
    B, S, D = A_x.shape
    F = B_w1.shape[1]
    assert B == 1 and D == 8 * LANES and S % T == 0 and F % FC == 0
    any_spec = pl.BlockSpec(memory_space=pl.ANY)
    out = pl.pallas_call(
        functools.partial(_kernel, T=T, R=R, FC=FC),
        grid=(S // T,),
        in_specs=[
            pl.BlockSpec((T, D), lambda i: (i, 0)),
            any_spec, any_spec, any_spec,
            pl.BlockSpec((1, F), lambda i: (0, 0)),
            any_spec,
            pl.BlockSpec((1, D), lambda i: (0, 0)),
        ],
        out_specs=pl.BlockSpec((T, D), lambda i: (i, 0)),
        out_shape=jax.ShapeDtypeStruct((S, D), A_x.dtype),
        scratch_shapes=[
            pltpu.VMEM((D, 3 * D), BF16),
            pltpu.VMEM((D, D), BF16),
            pltpu.VMEM((D, F), BF16),
            pltpu.VMEM((F, D), BF16),
            pltpu.VMEM((8, T, LANES), F32),
            pltpu.VMEM((2, 8, T + HALO, LANES), F32),
            pltpu.VMEM((2, 8, T + HALO, LANES), F32),
            pltpu.VMEM((T, D), BF16),
            pltpu.SemaphoreType.DMA((6,)),
        ],
        compiler_params=pltpu.CompilerParams(
            dimension_semantics=("arbitrary",),
            vmem_limit_bytes=100 * 1024 * 1024,
        ),
    )(A_x.reshape(S, D), A_wqkv, A_wo, B_w1, B_b1.reshape(1, F), B_w2, B_b2.reshape(1, D))
    return out.reshape(B, S, D)


@jax.jit
def pallas_interleave_layers__sliding_local_dilated__dense_activation_gelu__prompt_kernel(
    A_x: jax.Array,
    A_wqkv: jax.Array,
    A_wo: jax.Array,
    B_x: jax.Array,
    B_w1: jax.Array,
    B_b1: jax.Array,
    B_w2: jax.Array,
    B_b2: jax.Array,
):
    del B_x
    return _forward(A_x, A_wqkv, A_wo, B_w1, B_b1, B_w2, B_b2)
```

```python
import functools
import math

import jax
import jax.numpy as jnp
from jax import lax
import jax.experimental.pallas as pl
import jax.experimental.pallas.tpu as pltpu

H = 32
W = 8
DIL = 2
HALO = 16
LANES = 128
EPS = 1e-5
F32 = jnp.float32
BF16 = jnp.bfloat16


def _layernorm(x):
    m = jnp.mean(x, axis=-1, keepdims=True)
    xc = x - m
    v = jnp.mean(xc * xc, axis=-1, keepdims=True)
    return xc * lax.rsqrt(v + EPS)


def _gelu(x):
    c = math.sqrt(2.0 / math.pi)
    hx = 0.5 * x
    return hx + hx * jnp.tanh(x * (c + (c * 0.044715) * (x * x)))


def _butterfly(tiles, idx, axis, size, unit):
    tiles = list(tiles)
    for tb in (4, 2, 1):
        s = tb * unit
        m = (idx & s) == 0
        new = list(tiles)
        for g in range(8):
            if g & tb:
                continue
            x, y = tiles[g], tiles[g | tb]
            new[g] = jnp.where(m, x, pltpu.roll(y, s, axis))
            new[g | tb] = jnp.where(m, pltpu.roll(x, size - s, axis), y)
        tiles = new
    return tiles


def _permute_cols(w_ref, col0):
    rb = 32

    def body(r, carry):
        r0 = pl.multiple_of(r * rb, rb)
        tiles = [pltpu.bitcast(w_ref[pl.ds(r0, rb), pl.ds(col0 + LANES * g, LANES)], jnp.uint32)
                 for g in range(8)]
        lane = lax.broadcasted_iota(jnp.int32, tiles[0].shape, 1)
        tiles = _butterfly(tiles, lane, 1, LANES, 4)
        for g in range(8):
            w_ref[pl.ds(r0, rb), pl.ds(col0 + LANES * g, LANES)] = pltpu.bitcast(tiles[g], BF16)
        return carry

    lax.fori_loop(0, w_ref.shape[0] // rb, body, 0)


def _permute_rows(w_ref):
    def body(t, carry):
        a = t // 8
        n = t % 8
        r0 = pl.multiple_of(a * 32, 32)
        c0 = pl.multiple_of(n * LANES, LANES)
        tiles = [pltpu.bitcast(w_ref[pl.ds(r0 + LANES * g, 32), pl.ds(c0, LANES)], jnp.uint32)
                 for g in range(8)]
        row = lax.broadcasted_iota(jnp.int32, tiles[0].shape, 0)
        tiles = _butterfly(tiles, row, 0, 16, 2)
        for g in range(8):
            w_ref[pl.ds(r0 + LANES * g, 32), pl.ds(c0, LANES)] = pltpu.bitcast(tiles[g], BF16)
        return carry

    lax.fori_loop(0, 32, body, 0)


def _attn_rows(q_s, k_s, v_s, o_s, r0, R, pos0):
    lane = lax.broadcasted_iota(jnp.int32, (R, LANES), 1)
    m1 = (lane & 1) == 0
    m2 = (lane & 2) == 0
    q = [q_s[g, pl.ds(r0, R), :] for g in range(8)]
    logits = []
    for w in range(W):
        off = r0 + HALO - DIL * w
        acc = q[0] * k_s[0, pl.ds(off, R), :]
        for g in range(1, 8):
            acc = acc + q[g] * k_s[g, pl.ds(off, R), :]
        acc = acc + jnp.where(m1, pltpu.roll(acc, LANES - 1, 1), pltpu.roll(acc, 1, 1))
        acc = acc + jnp.where(m2, pltpu.roll(acc, LANES - 2, 1), pltpu.roll(acc, 2, 1))
        if pos0 is not None and w > 0:
            pos = pos0 + lax.broadcasted_iota(jnp.int32, (R, LANES), 0)
            acc = jnp.where(pos >= DIL * w, acc, -1e9)
        logits.append(acc)
    mx = logits[0]
    for w in range(1, W):
        mx = jnp.maximum(mx, logits[w])
    p = [jnp.exp2(l - mx) for l in logits]
    den = p[0]
    for w in range(1, W):
        den = den + p[w]
    inv = 1.0 / den
    p = [pw * inv for pw in p]
    for g in range(8):
        acc = p[0] * v_s[g, pl.ds(r0 + HALO, R), :]
        for w in range(1, W):
            acc = acc + p[w] * v_s[g, pl.ds(r0 + HALO - DIL * w, R), :]
        o_s[pl.ds(r0, R), pl.ds(LANES * g, LANES)] = acc.astype(BF16)


def _kernel(x_ref, wqkv_hbm, wo_hbm, w1_hbm, b1_ref, w2_hbm, b2_ref, out_ref,
            wqkv_s, wo_s, w1_s, w2_s, q_s, k_s, v_s, o_s, x_s, xn_s, sems, *, T, R, FC, LLOOP, FLOOP, WAIT_MID):
    i = pl.program_id(0)
    D = x_ref.shape[1]
    F = w1_s.shape[1]
    qscale = (D // H) ** -0.5 * math.log2(math.e)

    def cp_qkv(p):
        return pltpu.make_async_copy(wqkv_hbm.at[:, pl.ds(p * D, D)], wqkv_s.at[:, pl.ds(p * D, D)], sems.at[p])

    cp_wo = pltpu.make_async_copy(wo_hbm, wo_s, sems.at[3])
    cp_w1 = pltpu.make_async_copy(w1_hbm, w1_s, sems.at[4])
    cp_w2 = pltpu.make_async_copy(w2_hbm, w2_s, sems.at[5])

    @pl.when(i == 0)
    def _():
        for p in range(3):
            cp_qkv(p).start()
        cp_wo.start()
        cp_w1.start()
        cp_w2.start()
        k_s[:, :, pl.ds(T, HALO), :] = jnp.zeros((2, 8, HALO, LANES), F32)
        v_s[:, :, pl.ds(T, HALO), :] = jnp.zeros((2, 8, HALO, LANES), F32)
        for p in range(3):
            cp_qkv(p).wait()
            _permute_cols(wqkv_s, p * D)
        cp_wo.wait()
        _permute_rows(wo_s)
        if not WAIT_MID:
            cp_w1.wait()
            cp_w2.wait()

    x_s[...] = x_ref[...].astype(F32)

    def layer_body(layer, carry):
        x = x_s[...]
        kl = k_s.at[layer]
        vl = v_s.at[layer]
        kl[:, pl.ds(0, HALO), :] = kl[:, pl.ds(T, HALO), :]
        vl[:, pl.ds(0, HALO), :] = vl[:, pl.ds(T, HALO), :]
        xn = _layernorm(x).astype(BF16)
        q = jnp.dot(xn, wqkv_s[:, pl.ds(0, D)], preferred_element_type=F32) * qscale
        for g in range(8):
            q_s[g] = q[:, LANES * g:LANES * (g + 1)]
        k = jnp.dot(xn, wqkv_s[:, pl.ds(D, D)], preferred_element_type=F32)
        for g in range(8):
            kl[g, pl.ds(HALO, T), :] = k[:, LANES * g:LANES * (g + 1)]
        v = jnp.dot(xn, wqkv_s[:, pl.ds(2 * D, D)], preferred_element_type=F32)
        for g in range(8):
            vl[g, pl.ds(HALO, T), :] = v[:, LANES * g:LANES * (g + 1)]
        for c in range(T // R):
            _attn_rows(q_s, kl, vl, o_s, c * R, R, (i * T + c * R) if c * R < HALO else None)
        x = x + jnp.dot(o_s[...], wo_s[...], preferred_element_type=F32)

        if WAIT_MID:
            @pl.when(jnp.logical_and(i == 0, layer == 0))
            def _():
                cp_w1.wait()
                cp_w2.wait()

        xn = _layernorm(x).astype(BF16)
        x = x + b2_ref[...].astype(F32)
        if FLOOP:
            xn_s[...] = xn
            x_s[...] = x

            def fbody(c, carry):
                c0 = pl.multiple_of(c * FC, FC)
                h = jnp.dot(xn_s[...], w1_s[:, pl.ds(c0, FC)], preferred_element_type=F32)
                h = _gelu(h + b1_ref[:, pl.ds(c0, FC)].astype(F32)).astype(BF16)
                x_s[...] += jnp.dot(h, w2_s[pl.ds(c0, FC), :], preferred_element_type=F32)
                return carry

            lax.fori_loop(0, F // FC, fbody, 0)
        else:
            for c in range(F // FC):
                h = jnp.dot(xn, w1_s[:, pl.ds(c * FC, FC)], preferred_element_type=F32)
                h = _gelu(h + b1_ref[:, pl.ds(c * FC, FC)].astype(F32)).astype(BF16)
                x = x + jnp.dot(h, w2_s[pl.ds(c * FC, FC), :], preferred_element_type=F32)
            x_s[...] = x
        return carry

    if LLOOP:
        lax.fori_loop(0, 2, layer_body, 0)
    else:
        layer_body(0, 0)
        layer_body(1, 0)
    out_ref[...] = x_s[...].astype(out_ref.dtype)


def _forward(A_x, A_wqkv, A_wo, B_w1, B_b1, B_w2, B_b2, T=256, R=16, FC=512, LLOOP=True, FLOOP=False, WAIT_MID=True):
    B, S, D = A_x.shape
    F = B_w1.shape[1]
    assert B == 1 and D == 8 * LANES and S % T == 0 and F % FC == 0
    any_spec = pl.BlockSpec(memory_space=pl.ANY)
    out = pl.pallas_call(
        functools.partial(_kernel, T=T, R=R, FC=FC, LLOOP=LLOOP, FLOOP=FLOOP, WAIT_MID=WAIT_MID),
        grid=(S // T,),
        in_specs=[
            pl.BlockSpec((T, D), lambda i: (i, 0)),
            any_spec, any_spec, any_spec,
            pl.BlockSpec((1, F), lambda i: (0, 0)),
            any_spec,
            pl.BlockSpec((1, D), lambda i: (0, 0)),
        ],
        out_specs=pl.BlockSpec((T, D), lambda i: (i, 0)),
        out_shape=jax.ShapeDtypeStruct((S, D), A_x.dtype),
        scratch_shapes=[
            pltpu.VMEM((D, 3 * D), BF16),
            pltpu.VMEM((D, D), BF16),
            pltpu.VMEM((D, F), BF16),
            pltpu.VMEM((F, D), BF16),
            pltpu.VMEM((8, T, LANES), F32),
            pltpu.VMEM((2, 8, T + HALO, LANES), F32),
            pltpu.VMEM((2, 8, T + HALO, LANES), F32),
            pltpu.VMEM((T, D), BF16),
            pltpu.VMEM((T, D), F32),
            pltpu.VMEM((T, D), BF16),
            pltpu.SemaphoreType.DMA((6,)),
        ],
        compiler_params=pltpu.CompilerParams(
            dimension_semantics=("arbitrary",),
            vmem_limit_bytes=100 * 1024 * 1024,
        ),
    )(A_x.reshape(S, D), A_wqkv, A_wo, B_w1, B_b1.reshape(1, F), B_w2, B_b2.reshape(1, D))
    return out.reshape(B, S, D)


@jax.jit
def pallas_interleave_layers__sliding_local_dilated__dense_activation_gelu__prompt_kernel(
    A_x: jax.Array,
    A_wqkv: jax.Array,
    A_wo: jax.Array,
    B_x: jax.Array,
    B_w1: jax.Array,
    B_b1: jax.Array,
    B_w2: jax.Array,
    B_b2: jax.Array,
):
    del B_x
    return _forward(A_x, A_wqkv, A_wo, B_w1, B_b1, B_w2, B_b2)
```

```python
import functools
import math

import jax
import jax.numpy as jnp
from jax import lax
import jax.experimental.pallas as pl
import jax.experimental.pallas.tpu as pltpu

H = 32
W = 8
LANES = 128
G = 8
EXT = 16 * (W - 1)
EPS = 1e-5
F32 = jnp.float32
BF16 = jnp.bfloat16
U32 = jnp.uint32


def _layernorm(x):
    m = jnp.mean(x, axis=-1, keepdims=True)
    xc = x - m
    v = jnp.mean(xc * xc, axis=-1, keepdims=True)
    return xc * lax.rsqrt(v + EPS)


def _gelu(x):
    c = math.sqrt(2.0 / math.pi)
    hx = 0.5 * x
    return hx + hx * jnp.tanh(x * (c + (c * 0.044715) * (x * x)))


def _barrel(tiles, b):
    for t in (1, 2, 4):
        m = (b & t) != 0
        tiles = [jnp.where(m, tiles[(j + t) % 8], tiles[j]) for j in range(8)]
    return tiles


def _permute_cols_block(src_ref, w_ref, r0, rb, col0):
    tiles = [pltpu.bitcast(src_ref[pl.ds(r0, rb), pl.ds(col0 + LANES * g, LANES)], U32) for g in range(G)]
    b = (lax.broadcasted_iota(jnp.int32, tiles[0].shape, 1) >> 2) & 7
    tiles = [jnp.where(b > g, pltpu.roll(tiles[g], LANES - 32, 1), tiles[g]) if g < 7 else tiles[g]
             for g in range(G)]
    tiles = _barrel(tiles, b)
    for j in range(G):
        t = pltpu.roll(tiles[j], 4 * j, 1) if j else tiles[j]
        w_ref[pl.ds(r0, rb), pl.ds(col0 + LANES * j, LANES)] = pltpu.bitcast(t, BF16)


def _permute_rows_block(src_ref, w_ref, r0, c0, cb):
    tiles = [pltpu.bitcast(src_ref[pl.ds(r0 + LANES * g, 32), pl.ds(c0, cb)], U32) for g in range(G)]
    b = lax.broadcasted_iota(jnp.int32, tiles[0].shape, 0) >> 1
    tiles = _barrel(tiles, b)
    for j in range(G):
        t = pltpu.roll(tiles[j], 2 * j, 0) if j else tiles[j]
        w_ref[pl.ds(r0 + LANES * j, 32), pl.ds(c0, cb)] = pltpu.bitcast(t, BF16)


def _transpose8(tiles):
    sub = lax.broadcasted_iota(jnp.int32, tiles[0].shape, 0)
    for s in (4, 2, 1):
        m = (sub & s) == 0
        new = list(tiles)
        for g in range(8):
            if g & s:
                continue
            x, y = tiles[g], tiles[g | s]
            new[g] = jnp.where(m, x, pltpu.roll(y, s, 0))
            new[g | s] = jnp.where(m, pltpu.roll(x, 8 - s, 0), y)
        tiles = new
    return tiles


def _load_rows_permuted(x_ref, row0, T):
    blocks = []
    for hi in range(T // 128):
        tiles = [pltpu.bitcast(x_ref[pl.ds(row0 + u * (T // 8) + 16 * hi, 16), :], U32) for u in range(8)]
        blocks += [pltpu.bitcast(t, BF16) for t in _transpose8(tiles)]
    return jnp.concatenate(blocks, axis=0)


def _store_rows_unpermuted(x_ref, row0, T, val):
    for hi in range(T // 128):
        tiles = [pltpu.bitcast(val[128 * hi + 16 * t:128 * hi + 16 * (t + 1), :], U32) for t in range(8)]
        tiles = _transpose8(tiles)
        for u in range(8):
            x_ref[pl.ds(row0 + u * (T // 8) + 16 * hi, 16), :] = pltpu.bitcast(tiles[u], BF16)


def _store_kv(val, kv_s, halo_s, T):
    first = lax.broadcasted_iota(jnp.int32, (8, LANES), 0) < 2
    for g in range(G):
        col = val[:, LANES * g:LANES * (g + 1)]
        kv_s[g, pl.ds(EXT, T), :] = col
        for e in range(W - 1):
            r = T - EXT + 16 * e
            lo = pltpu.roll(col[r:r + 8], 2, 0)
            hi = pltpu.roll(col[r + 8:r + 16], 2, 0)
            kv_s[g, pl.ds(16 * e, 8), :] = jnp.where(first, halo_s[g, pl.ds(8 * e, 8), :], lo)
            kv_s[g, pl.ds(16 * e + 8, 8), :] = jnp.where(first, lo, hi)
            halo_s[g, pl.ds(8 * e, 8), :] = hi


def _attn_block(q_s, k_s, v_s, o_s, i, invalid):
    R = 16
    r0 = R * i
    lane = lax.broadcasted_iota(jnp.int32, (R, LANES), 1)
    m1 = (lane & 1) == 0
    m2 = (lane & 2) == 0
    q = [q_s[g, pl.ds(r0, R), :] for g in range(G)]
    logits = []
    for w in range(W):
        off = EXT + r0 - R * w
        acc = q[0] * k_s[0, pl.ds(off, R), :]
        for g in range(1, G):
            acc = acc + q[g] * k_s[g, pl.ds(off, R), :]
        acc = acc + jnp.where(m1, pltpu.roll(acc, LANES - 1, 1), pltpu.roll(acc, 1, 1))
        acc = acc + jnp.where(m2, pltpu.roll(acc, LANES - 2, 1), pltpu.roll(acc, 2, 1))
        if i < w:
            acc = jnp.where(invalid, -1e9, acc)
        logits.append(acc)
    mx = logits[0]
    for w in range(1, W):
        mx = jnp.maximum(mx, logits[w])
    p = [jnp.exp2(l - mx) for l in logits]
    den = p[0]
    for w in range(1, W):
        den = den + p[w]
    inv = 1.0 / den
    p = [pw * inv for pw in p]
    for g in range(G):
        acc = p[0] * v_s[g, pl.ds(EXT + r0, R), :]
        for w in range(1, W):
            acc = acc + p[w] * v_s[g, pl.ds(EXT + r0 - R * w, R), :]
        o_s[pl.ds(r0, R), pl.ds(LANES * g, LANES)] = acc.astype(BF16)


def _kernel(x_hbm, wqkv_hbm, wo_hbm, w1_hbm, b1_ref, w2_hbm, b2_ref, out_hbm,
            wqkv_r, wo_r, wqkv_s, wo_s, w1_s, w2_s, xio_s, xm_s, xn_s, q_s, k_s, v_s, hk_s, hv_s, o_s,
            wsem, xsem, osem, *, T, FC, LAG, ORDER, TLOOP):
    S, D = xio_s.shape
    F = w1_s.shape[1]
    NT = S // T
    NC = F // FC
    qscale = (D // H) ** -0.5 * math.log2(math.e)

    def cp_qkv(p):
        return pltpu.make_async_copy(wqkv_hbm.at[:, pl.ds(p * D, D)], wqkv_r.at[:, pl.ds(p * D, D)], wsem.at[p])

    cp_wo = pltpu.make_async_copy(wo_hbm, wo_r, wsem.at[3])
    cp_w1 = pltpu.make_async_copy(w1_hbm, w1_s, wsem.at[4])
    cp_w2 = pltpu.make_async_copy(w2_hbm, w2_s, wsem.at[5])

    def rows(t):
        return pl.ds(pl.multiple_of(t * T, T), T)

    def cp_x(t):
        return pltpu.make_async_copy(x_hbm.at[rows(t)], xio_s.at[rows(t)], xsem.at[t])

    def cp_out(t):
        return pltpu.make_async_copy(xio_s.at[rows(t)], out_hbm.at[rows(t)], osem.at[t])

    def dot(a, b):
        return jnp.dot(a, b, preferred_element_type=F32)

    def step(na, nf, order):
        st = {}
        if na is not None:
            ta = na % NT
            sa = na % (LAG + 1)
        if nf is not None:
            tf = nf % NT
            sf = nf % (LAG + 1)
        for op in order:
            if op[0] == "f":
                if nf is None:
                    continue
            elif na is None:
                continue
            if op == "ln1":
                st["x"] = _load_rows_permuted(xio_s, pl.multiple_of(ta * T, T), T).astype(F32)
                st["xn"] = _layernorm(st["x"]).astype(BF16)
            elif op == "q":
                q = dot(st["xn"], wqkv_s[:, pl.ds(0, D)]) * qscale
                for g in range(G):
                    q_s[g] = q[:, LANES * g:LANES * (g + 1)]
            elif op == "k":
                _store_kv(dot(st["xn"], wqkv_s[:, pl.ds(D, D)]), k_s, hk_s, T)
            elif op == "v":
                _store_kv(dot(st["xn"], wqkv_s[:, pl.ds(2 * D, D)]), v_s, hv_s, T)
            elif op.startswith("att"):
                part, nparts = (int(op[3]), int(op[4])) if len(op) > 3 else (0, 1)
                nb = T // 16 // nparts
                row = lax.broadcasted_iota(jnp.int32, (16, LANES), 0)
                invalid = row < jnp.where(ta == 0, 2, 0)
                for i in range(part * nb, (part + 1) * nb):
                    _attn_block(q_s, k_s, v_s, o_s, i, invalid)
            elif op == "wo":
                st["x"] = st["x"] + dot(o_s[...], wo_s[...])
            elif op == "ln2":
                xn_s[sa] = _layernorm(st["x"]).astype(BF16)
                xm_s[sa] = st["x"] + b2_ref[...].astype(F32)
            elif op == "fbeg":
                st["fxn"] = xn_s[sf]
                st["facc"] = xm_s[sf]
            elif op == "fend":
                _store_rows_unpermuted(xio_s, pl.multiple_of(tf * T, T), T, st["facc"].astype(BF16))
            else:
                c = int(op[1:])
                h = dot(st["fxn"], w1_s[:, pl.ds(c * FC, FC)])
                h = _gelu(h + b1_ref[:, pl.ds(c * FC, FC)].astype(F32)).astype(BF16)
                st["facc"] = st["facc"] + dot(h, w2_s[pl.ds(c * FC, FC), :])

    order = ORDER.split(",")
    assert sorted(int(o[1:]) for o in order if o[1:].isdigit()) == list(range(NC))

    cp_x(0).start()
    for p in range(3):
        cp_qkv(p).start()
    cp_wo.start()
    for t in range(1, LAG + 1):
        cp_x(t).start()
    cp_w1.start()
    cp_w2.start()
    for t in range(LAG + 1, NT):
        cp_x(t).start()
    hk_s[...] = jnp.zeros(hk_s.shape, F32)
    hv_s[...] = jnp.zeros(hv_s.shape, F32)
    RB = 128
    for p in range(3):
        cp_qkv(p).wait()

        def pbody(r, carry, p=p):
            for rr in range(0, RB, 32):
                _permute_cols_block(wqkv_r, wqkv_s, pl.multiple_of(r * RB, RB) + rr, 32, p * D)
            return carry

        lax.fori_loop(0, D // RB, pbody, 0)
    cp_wo.wait()

    def rbody(n, carry):
        for a in range(4):
            _permute_rows_block(wo_r, wo_s, 32 * a, pl.multiple_of(n * LANES, LANES), LANES)
        return carry

    lax.fori_loop(0, G, rbody, 0)

    def head(n, carry):
        cp_x(n).wait()
        step(n, None, order)
        return carry

    lax.fori_loop(0, LAG, head, 0)
    cp_w1.wait()
    cp_w2.wait()

    def steady(n, carry):
        @pl.when(n < NT)
        def _():
            cp_x(n).wait()

        step(n, n - LAG, order)

        @pl.when(n - LAG >= NT)
        def _():
            cp_out(n - LAG - NT).start()

        return carry

    lax.fori_loop(LAG, 2 * NT, steady, 0)

    def tail(n, carry):
        if TLOOP:
            sf = n % (LAG + 1)

            def chunk(c, carry):
                c0 = pl.multiple_of(c * FC, FC)
                h = dot(xn_s[sf], w1_s[:, pl.ds(c0, FC)])
                h = _gelu(h + b1_ref[:, pl.ds(c0, FC)].astype(F32)).astype(BF16)
                xm_s[sf] += dot(h, w2_s[pl.ds(c0, FC), :])
                return carry

            lax.fori_loop(0, NC, chunk, 0)
            step(None, n, ["fbeg", "fend"])
        else:
            step(None, n, order)
        cp_out(n - NT).start()
        return carry

    lax.fori_loop(2 * NT - LAG, 2 * NT, tail, 0)
    for t in range(NT):
        cp_out(t).wait()


def _forward(A_x, A_wqkv, A_wo, B_w1, B_b1, B_w2, B_b2, T=256, FC=512, LAG=2, TLOOP=True,
             ORDER="fbeg,ln1,f0,f1,q,k,v,att,f2,f3,wo,ln2,f4,f5,f6,fend"):
    B, S, D = A_x.shape
    F = B_w1.shape[1]
    assert B == 1 and D == G * LANES and S % T == 0 and F % FC == 0 and T % 128 == 0 and LAG < S // T
    any_spec = pl.BlockSpec(memory_space=pl.ANY)
    vmem_spec = pl.BlockSpec(memory_space=pltpu.VMEM)
    out = pl.pallas_call(
        functools.partial(_kernel, T=T, FC=FC, LAG=LAG, ORDER=ORDER, TLOOP=TLOOP),
        in_specs=[any_spec, any_spec, any_spec, any_spec, vmem_spec, any_spec, vmem_spec],
        out_specs=any_spec,
        out_shape=jax.ShapeDtypeStruct((S, D), A_x.dtype),
        scratch_shapes=[
            pltpu.VMEM((D, 3 * D), BF16),
            pltpu.VMEM((D, D), BF16),
            pltpu.VMEM((D, 3 * D), BF16),
            pltpu.VMEM((D, D), BF16),
            pltpu.VMEM((D, F), BF16),
            pltpu.VMEM((F, D), BF16),
            pltpu.VMEM((S, D), BF16),
            pltpu.VMEM((LAG + 1, T, D), F32),
            pltpu.VMEM((LAG + 1, T, D), BF16),
            pltpu.VMEM((G, T, LANES), F32),
            pltpu.VMEM((G, T + EXT, LANES), F32),
            pltpu.VMEM((G, T + EXT, LANES), F32),
            pltpu.VMEM((G, EXT // 2, LANES), F32),
            pltpu.VMEM((G, EXT // 2, LANES), F32),
            pltpu.VMEM((T, D), BF16),
            pltpu.SemaphoreType.DMA((6,)),
            pltpu.SemaphoreType.DMA((S // T,)),
            pltpu.SemaphoreType.DMA((S // T,)),
        ],
        compiler_params=pltpu.CompilerParams(vmem_limit_bytes=100 * 1024 * 1024),
    )(A_x.reshape(S, D), A_wqkv, A_wo, B_w1, B_b1.reshape(1, F), B_w2, B_b2.reshape(1, D))
    return out.reshape(B, S, D)


@jax.jit
def pallas_interleave_layers__sliding_local_dilated__dense_activation_gelu__prompt_kernel(
    A_x: jax.Array,
    A_wqkv: jax.Array,
    A_wo: jax.Array,
    B_x: jax.Array,
    B_w1: jax.Array,
    B_b1: jax.Array,
    B_w2: jax.Array,
    B_b2: jax.Array,
):
    del B_x
    return _forward(A_x, A_wqkv, A_wo, B_w1, B_b1, B_w2, B_b2)
```

```python
import functools
import math

import jax
import jax.numpy as jnp
from jax import lax
import jax.experimental.pallas as pl
import jax.experimental.pallas.tpu as pltpu

H = 32
W = 8
LANES = 128
G = 8
EXT = 16 * (W - 1)
EPS = 1e-5
F32 = jnp.float32
BF16 = jnp.bfloat16
U32 = jnp.uint32


def _layernorm(x):
    m = jnp.mean(x, axis=-1, keepdims=True)
    xc = x - m
    v = jnp.mean(xc * xc, axis=-1, keepdims=True)
    return xc * lax.rsqrt(v + EPS)


def _gelu(x):
    c = math.sqrt(2.0 / math.pi)
    hx = 0.5 * x
    return hx + hx * jnp.tanh(x * (c + (c * 0.044715) * (x * x)))


def _pack(x):
    return pltpu.bitcast(x.astype(BF16), U32)


def _unpack(u):
    return pltpu.bitcast(u, BF16)


def _barrel(tiles, b):
    for t in (1, 2, 4):
        m = (b & t) != 0
        tiles = [jnp.where(m, tiles[(j + t) % 8], tiles[j]) for j in range(8)]
    return tiles


def _permute_cols_block(src_ref, w_ref, h0, hb):
    rows = pl.ds(pl.multiple_of(2 * h0, 2 * hb), 2 * hb)
    tiles = [_pack(src_ref[rows, pl.ds(LANES * g, LANES)]) for g in range(G)]
    b = (lax.broadcasted_iota(jnp.int32, tiles[0].shape, 1) >> 2) & 7
    tiles = _barrel(tiles, b)
    for j in range(G):
        t = tiles[j]
        if j:
            t = jnp.where(b >= j, pltpu.roll(t, 4 * j, 1), pltpu.roll(t, LANES - 32 + 4 * j, 1))
        w_ref[pl.ds(pl.multiple_of(h0, hb), hb), pl.ds(LANES * j, LANES)] = t


def _permute_rows_block(src_ref, w_ref, r0, n):
    cols = pl.ds(pl.multiple_of(n * LANES, LANES), LANES)
    tiles = [_pack(src_ref[pl.ds(r0 + LANES * g, 32), cols]) for g in range(G)]
    b = lax.broadcasted_iota(jnp.int32, tiles[0].shape, 0) >> 1
    tiles = _barrel(tiles, b)
    for j in range(G):
        t = pltpu.roll(tiles[j], 2 * j, 0) if j else tiles[j]
        w_ref[pl.ds((r0 + LANES * j) // 2, 16), cols] = t


def _transpose8(tiles):
    sub = lax.broadcasted_iota(jnp.int32, tiles[0].shape, 0)
    for s in (4, 2, 1):
        m = (sub & s) == 0
        new = list(tiles)
        for g in range(8):
            if g & s:
                continue
            x, y = tiles[g], tiles[g | s]
            new[g] = jnp.where(m, x, pltpu.roll(y, s, 0))
            new[g | s] = jnp.where(m, pltpu.roll(x, 8 - s, 0), y)
        tiles = new
    return tiles


def _load_rows_permuted(x_ref, row0, T):
    blocks = []
    for hi in range(T // 128):
        blocks += _transpose8([_pack(x_ref[pl.ds(row0 + u * (T // 8) + 16 * hi, 16), :]) for u in range(8)])
    return jnp.concatenate(blocks, axis=0)


def _store_rows_unpermuted(x_ref, row0, T, val):
    for hi in range(T // 128):
        tiles = _transpose8([_pack(val[128 * hi + 16 * t:128 * hi + 16 * (t + 1), :]) for t in range(8)])
        for u in range(8):
            x_ref[pl.ds(row0 + u * (T // 8) + 16 * hi, 16), :] = _unpack(tiles[u])


def _store_kv(val, kv_s, halo_s, T):
    first = lax.broadcasted_iota(jnp.int32, (8, LANES), 0) < 2
    for g in range(G):
        col = val[:, LANES * g:LANES * (g + 1)]
        kv_s[g, pl.ds(EXT, T), :] = col
        for e in range(W - 1):
            r = T - EXT + 16 * e
            lo = pltpu.roll(col[r:r + 8], 2, 0)
            hi = pltpu.roll(col[r + 8:r + 16], 2, 0)
            kv_s[g, pl.ds(16 * e, 8), :] = jnp.where(first, halo_s[g, pl.ds(8 * e, 8), :], lo)
            kv_s[g, pl.ds(16 * e + 8, 8), :] = jnp.where(first, lo, hi)
            halo_s[g, pl.ds(8 * e, 8), :] = hi


def _attn_probs(q_s, k_s, i, invalid):
    R = 16
    r0 = R * i
    lane = lax.broadcasted_iota(jnp.int32, (R, LANES), 1)
    m1 = (lane & 1) == 0
    m2 = (lane & 2) == 0
    q = [q_s[g, pl.ds(r0, R), :] for g in range(G)]
    logits = []
    for w in range(W):
        off = EXT + r0 - R * w
        acc = q[0] * k_s[0, pl.ds(off, R), :]
        for g in range(1, G):
            acc = acc + q[g] * k_s[g, pl.ds(off, R), :]
        acc = acc + jnp.where(m1, pltpu.roll(acc, LANES - 1, 1), pltpu.roll(acc, 1, 1))
        acc = acc + jnp.where(m2, pltpu.roll(acc, LANES - 2, 1), pltpu.roll(acc, 2, 1))
        if i < w:
            acc = jnp.where(invalid, -1e9, acc)
        logits.append(acc)
    mx = logits[0]
    for w in range(1, W):
        mx = jnp.maximum(mx, logits[w])
    p = [jnp.exp2(l - mx) for l in logits]
    den = p[0]
    for w in range(1, W):
        den = den + p[w]
    return p, 1.0 / den


def _attn_values(p, inv, v_s, o_s, i):
    R = 16
    r0 = R * i
    for g in range(G):
        acc = p[0] * v_s[g, pl.ds(EXT + r0, R), :]
        for w in range(1, W):
            acc = acc + p[w] * v_s[g, pl.ds(EXT + r0 - R * w, R), :]
        o_s[pl.ds(r0 // 2, R // 2), pl.ds(LANES * g, LANES)] = _pack(acc * inv)


def _kernel(x_hbm, wqkv_hbm, wo_hbm, w1_hbm, b1_ref, w2_hbm, b2_ref, out_hbm,
            wqkv_r, wo_r, wa_s, w1_s, w2_s, xio_s, xp_s, x1_s, xm_s, xn_s, q_s, k_s, v_s, hk_s, hv_s, o_s,
            wsem, xsem, osem, *, T, FC, LAG, ORDER, O_HEAD, TLOOP, KCH, PRB):
    S, D = xio_s.shape
    F = w1_s.shape[1]
    NT = S // T
    NC = F // FC
    qscale = (D // H) ** -0.5 * math.log2(math.e)

    RC = D // KCH

    def cp_qkv(p, c):
        r = pl.ds(pl.multiple_of(c * RC, RC), RC)
        cols = pl.ds(pl.multiple_of(p * D, D), D)
        return pltpu.make_async_copy(wqkv_hbm.at[r, cols], wqkv_r.at[p, r], wsem.at[3 + p * KCH + c])

    def perm_cols(p0, p1):
        def body(t, carry):
            p, c = t // KCH, t % KCH
            cp_qkv(p, c).wait()
            for rr in range(0, RC, PRB):
                _permute_cols_block(wqkv_r.at[p], wa_s.at[p], c * (RC // 2) + rr // 2, PRB // 2)
            return carry

        lax.fori_loop(p0 * KCH, p1 * KCH, body, 0)

    def perm_rows():
        def body(n, carry):
            for a in range(4):
                _permute_rows_block(wo_r, wa_s.at[3], 32 * a, n)
            return carry

        cp_wo.wait()
        lax.fori_loop(0, G, body, 0)

    cp_wo = pltpu.make_async_copy(wo_hbm, wo_r, wsem.at[0])
    cp_w1 = pltpu.make_async_copy(w1_hbm, w1_s, wsem.at[1])
    cp_w2 = pltpu.make_async_copy(w2_hbm, w2_s, wsem.at[2])

    def rows(t):
        return pl.ds(pl.multiple_of(t * T, T), T)

    def cp_x(t):
        return pltpu.make_async_copy(x_hbm.at[rows(t)], xio_s.at[rows(t)], xsem.at[t])

    def cp_out(t):
        return pltpu.make_async_copy(xio_s.at[rows(t)], out_hbm.at[rows(t)], osem.at[t])

    def dot(a, b):
        return jnp.dot(a, b, preferred_element_type=F32)

    def wcat(p):
        return _unpack(wa_s[p])

    def xperm(n):
        xp = _load_rows_permuted(xio_s, pl.multiple_of((n % NT) * T, T), T)
        xp_s[n % 2] = xp
        toks = []
        for hi in range(T // 128):
            for g in range(G):
                t = xp[64 * hi:64 * (hi + 1), LANES * g:LANES * (g + 1)]
                toks.append(pltpu.bitcast(t[0:16] | t[16:32] | t[32:48] | t[48:64], F32))
        return toks

    def tie(x, never, tok):
        if tok is None:
            return x
        x0 = jnp.where(never, tok, x[:, :LANES])
        return x0 if x.shape[1] == LANES else jnp.concatenate([x0, x[:, LANES:]], axis=1)

    def ln1(n, never=None, toks=None):
        for i in range(T // 16):
            r = pl.ds(8 * i, 8)
            x = tie(_unpack(xp_s[n % 2, r, :]).astype(F32), never, toks and toks[i])
            x1_s[r, :] = _pack(_layernorm(x))

    def ln2(n, never=None, toks=None):
        s = n % (LAG + 1)
        for i in range(T // 16):
            x = tie(xm_s[s, pl.ds(16 * i, 16), :], never, toks and toks[i])
            xn_s[s, pl.ds(8 * i, 8), :] = _pack(_layernorm(x))

    def step(na, nf, order):
        st = {}
        if na is not None:
            ta = na % NT
            sa = na % (LAG + 1)
            never = lax.broadcasted_iota(jnp.int32, (16, LANES), 0) < jnp.minimum(na, 0)
        if nf is not None:
            tf = nf % NT
            sf = nf % (LAG + 1)

        def tokens(op, count=T // 16):
            if ":" not in op:
                return None
            cols = []
            for src in op.split(":")[1].split("+"):
                if src not in st:
                    return None
                cols += [(st[src], j) for j in range(st[src].shape[1] // LANES)]
            nb = T // 16
            out = []
            for i in range(count):
                pos = i * len(cols) * nb // count
                val, j = cols[pos // nb]
                r = 16 * (pos % nb)
                out.append(val[r:r + 16, LANES * j:LANES * (j + 1)])
            return out

        def pull(val, spec):
            if spec is None or spec.split(".")[0] not in st:
                return val
            name, a, b = spec.split(".")
            toks = st[name][int(a):int(b)]
            nc, nb = val.shape[1] // LANES, T // 16
            at = {divmod((2 * i + 1) * nc * nb // (2 * len(toks)), nb): t for i, t in enumerate(toks)}
            cols = []
            for j in range(nc):
                col = val[:, LANES * j:LANES * (j + 1)]
                if any(jj == j for jj, _ in at):
                    col = jnp.concatenate([tie(col[16 * r:16 * (r + 1)], never, at.get((j, r)))
                                           for r in range(nb)], axis=0)
                cols.append(col)
            return jnp.concatenate(cols, axis=1)

        for op in order:
            op, *specs = op.split("/")
            specs = dict(sp.split("<") for sp in specs)
            if op[0] == "f":
                if nf is None:
                    continue
            elif na is None:
                continue
            if op == "late":
                @pl.when(na == 0)
                def _():
                    perm_cols(2, 3)
                    perm_rows()
            elif op == "xwait":
                cp_x(na + 1).wait()
            elif op == "xp":
                st["xp"] = xperm(na + 1)
            elif op.startswith("ln1"):
                ln1(na + 1, never, tokens(op))
            elif op == "q":
                st["q"] = pull(dot(_unpack(x1_s[...]), wcat(0)), specs.get("y"))
                q = st["q"] * qscale
                for g in range(G):
                    q_s[g] = q[:, LANES * g:LANES * (g + 1)]
            elif op == "k":
                st["k"] = pull(dot(_unpack(x1_s[...]), wcat(1)), specs.get("y"))
                _store_kv(st["k"], k_s, hk_s, T)
            elif op == "v":
                st["v"] = pull(dot(_unpack(x1_s[...]), wcat(2)), specs.get("y"))
                _store_kv(st["v"], v_s, hv_s, T)
            elif op == "qk":
                row = lax.broadcasted_iota(jnp.int32, (16, LANES), 0)
                invalid = row < jnp.where(ta == 0, 2, 0)
                st["p"] = [_attn_probs(q_s, k_s, i, invalid) for i in range(T // 16)]
                st["sm"] = [inv for _, inv in st["p"]]
            elif op == "pv":
                for i in range(T // 16):
                    _attn_values(*st["p"][i], v_s, o_s, i)
            elif op == "wo":
                st["wo"] = _unpack(xp_s[na % 2]).astype(F32) + pull(dot(_unpack(o_s[...]), wcat(3)), specs.get("y"))
                xm_s[sa] = st["wo"]
            elif op.startswith("ln2"):
                ln2(na + LAG, never, tokens(op))
            elif op == "fbeg":
                st["fxn"] = _unpack(xn_s[sf])
                st["facc"] = xm_s[sf] + b2_ref[...].astype(F32)
            elif op == "fend":
                _store_rows_unpermuted(xio_s, pl.multiple_of(tf * T, T), T, st["facc"])
            else:
                c = int(op[1:])
                h = st[f"h{c}"] = pull(dot(st["fxn"], w1_s[:, pl.ds(c * FC, FC)]), specs.get("h"))
                h = _gelu(h + b1_ref[:, pl.ds(c * FC, FC)].astype(F32)).astype(BF16)
                st[f"y{c}"] = pull(dot(h, w2_s[pl.ds(c * FC, FC), :]), specs.get("y"))
                st[f"z{c}"] = st["facc"] = st["facc"] + st[f"y{c}"]

    order = ORDER.split(",")
    assert sorted(int(o[1]) for o in order if o[0] == "f" and o[1].isdigit()) == list(range(NC))

    cp_x(0).start()
    for p in range(3):
        for c in range(KCH):
            cp_qkv(p, c).start()
    cp_wo.start()
    for t in range(1, LAG + 2):
        cp_x(t).start()
    cp_w1.start()
    cp_w2.start()
    for t in range(LAG + 2, NT):
        cp_x(t).start()
    hk_s[...] = jnp.zeros(hk_s.shape, F32)
    hv_s[...] = jnp.zeros(hv_s.shape, F32)
    cp_x(0).wait()
    xperm(0)

    def ln_first(i, carry):
        r = pl.ds(pl.multiple_of(i * 32, 32), 32)
        x1_s[r, :] = _pack(_layernorm(_unpack(xp_s[0, r, :]).astype(F32)))
        xm_s[LAG, pl.ds(pl.multiple_of(i * 64, 64), 64), :] = jnp.zeros((64, D), F32)
        return carry

    lax.fori_loop(0, T // 64, ln_first, 0)

    if "late" in O_HEAD:
        perm_cols(0, 2)
    else:
        perm_cols(0, 3)
        perm_rows()

    def head(n, carry):
        step(n, None, O_HEAD.split(","))
        return carry

    lax.fori_loop(0, LAG, head, 0)
    cp_w1.wait()
    cp_w2.wait()

    def steady(n, carry):
        @pl.when(n + 1 < NT)
        def _():
            cp_x(n + 1).wait()

        step(n, n - LAG, order)

        @pl.when(n - LAG >= NT)
        def _():
            cp_out(n - LAG - NT).start()

        return carry

    lax.fori_loop(LAG, 2 * NT, steady, 0)
    ln2(2 * NT - 1)

    def tail(n, carry):
        if TLOOP:
            sf = n % (LAG + 1)

            def chunk(c, carry):
                c0 = pl.multiple_of(c * FC, FC)
                h = dot(_unpack(xn_s[sf]), w1_s[:, pl.ds(c0, FC)])
                h = _gelu(h + b1_ref[:, pl.ds(c0, FC)].astype(F32)).astype(BF16)
                xm_s[sf] += dot(h, w2_s[pl.ds(c0, FC), :])
                return carry

            lax.fori_loop(0, NC, chunk, 0)
            step(None, n, ["fbeg", "fend"])
        else:
            step(None, n, order)
        cp_out(n - NT).start()
        return carry

    lax.fori_loop(2 * NT - LAG, 2 * NT, tail, 0)
    for t in range(NT):
        cp_out(t).wait()


def _forward(A_x, A_wqkv, A_wo, B_w1, B_b1, B_w2, B_b2, T=256, FC=512, LAG=3, TLOOP=True, KCH=8, PRB=32,
             ORDER="fbeg,xp,k/y<xp.0.16,q,qk,f0,f1/h<sm.0.8/y<sm.8.16,v,pv,f2,f3,ln2:y2+y3,f4,f5,ln1:y4+y5,f6,fend,wo",
             O_HEAD="k,ln2:k,q,late,xwait,xp,qk,v,pv,wo,ln1"):
    B, S, D = A_x.shape
    F = B_w1.shape[1]
    assert B == 1 and D == G * LANES and S % T == 0 and F % FC == 0 and T % 128 == 0 and 2 <= LAG < S // T
    any_spec = pl.BlockSpec(memory_space=pl.ANY)
    vmem_spec = pl.BlockSpec(memory_space=pltpu.VMEM)
    out = pl.pallas_call(
        functools.partial(_kernel, T=T, FC=FC, LAG=LAG, ORDER=ORDER, O_HEAD=O_HEAD, TLOOP=TLOOP, KCH=KCH, PRB=PRB),
        in_specs=[any_spec, any_spec, any_spec, any_spec, vmem_spec, any_spec, vmem_spec],
        out_specs=any_spec,
        out_shape=jax.ShapeDtypeStruct((S, D), A_x.dtype),
        scratch_shapes=[
            pltpu.VMEM((3, D, D), BF16),
            pltpu.VMEM((D, D), BF16),
            pltpu.VMEM((4, D // 2, D), U32),
            pltpu.VMEM((D, F), BF16),
            pltpu.VMEM((F, D), BF16),
            pltpu.VMEM((S, D), BF16),
            pltpu.VMEM((2, T // 2, D), U32),
            pltpu.VMEM((T // 2, D), U32),
            pltpu.VMEM((LAG + 1, T, D), F32),
            pltpu.VMEM((LAG + 1, T // 2, D), U32),
            pltpu.VMEM((G, T, LANES), F32),
            pltpu.VMEM((G, T + EXT, LANES), F32),
            pltpu.VMEM((G, T + EXT, LANES), F32),
            pltpu.VMEM((G, EXT // 2, LANES), F32),
            pltpu.VMEM((G, EXT // 2, LANES), F32),
            pltpu.VMEM((T // 2, D), U32),
            pltpu.SemaphoreType.DMA((3 + 3 * KCH,)),
            pltpu.SemaphoreType.DMA((S // T,)),
            pltpu.SemaphoreType.DMA((S // T,)),
        ],
        compiler_params=pltpu.CompilerParams(vmem_limit_bytes=100 * 1024 * 1024),
    )(A_x.reshape(S, D), A_wqkv, A_wo, B_w1, B_b1.reshape(1, F), B_w2, B_b2.reshape(1, D))
    return out.reshape(B, S, D)


@jax.jit
def pallas_interleave_layers__sliding_local_dilated__dense_activation_gelu__prompt_kernel(
    A_x: jax.Array,
    A_wqkv: jax.Array,
    A_wo: jax.Array,
    B_x: jax.Array,
    B_w1: jax.Array,
    B_b1: jax.Array,
    B_w2: jax.Array,
    B_b2: jax.Array,
):
    del B_x
    return _forward(A_x, A_wqkv, A_wo, B_w1, B_b1, B_w2, B_b2)
```

```python
import functools
import math

import jax
import jax.numpy as jnp
from jax import lax
import jax.experimental.pallas as pl
import jax.experimental.pallas.tpu as pltpu

H = 32
W = 8
LANES = 128
G = 8
EXT = 16 * (W - 1)
EPS = 1e-5
F32 = jnp.float32
BF16 = jnp.bfloat16
U32 = jnp.uint32


def _layernorm(x):
    m = jnp.mean(x, axis=-1, keepdims=True)
    xc = x - m
    v = jnp.mean(xc * xc, axis=-1, keepdims=True)
    return xc * lax.rsqrt(v + EPS)


def _gelu(x):
    c = math.sqrt(2.0 / math.pi)
    hx = 0.5 * x
    return hx + hx * jnp.tanh(x * (c + (c * 0.044715) * (x * x)))


def _pack(x):
    return pltpu.bitcast(x.astype(BF16), U32)


def _unpack(u):
    return pltpu.bitcast(u, BF16)


def _barrel(tiles, b):
    for t in (1, 2, 4):
        m = (b & t) != 0
        tiles = [jnp.where(m, tiles[(j + t) % 8], tiles[j]) for j in range(8)]
    return tiles


def _permute_cols_block(src_ref, w_ref, h0, hb):
    rows = pl.ds(pl.multiple_of(2 * h0, 2 * hb), 2 * hb)
    tiles = [_pack(src_ref[rows, pl.ds(LANES * g, LANES)]) for g in range(G)]
    b = (lax.broadcasted_iota(jnp.int32, tiles[0].shape, 1) >> 2) & 7
    tiles = _barrel(tiles, b)
    for j in range(G):
        t = tiles[j]
        if j:
            t = jnp.where(b >= j, pltpu.roll(t, 4 * j, 1), pltpu.roll(t, LANES - 32 + 4 * j, 1))
        w_ref[pl.ds(pl.multiple_of(h0, hb), hb), pl.ds(LANES * j, LANES)] = t


def _permute_rows_block(src_ref, w_ref, r0, n):
    cols = pl.ds(pl.multiple_of(n * LANES, LANES), LANES)
    tiles = [_pack(src_ref[pl.ds(r0 + LANES * g, 32), cols]) for g in range(G)]
    b = lax.broadcasted_iota(jnp.int32, tiles[0].shape, 0) >> 1
    tiles = _barrel(tiles, b)
    for j in range(G):
        t = pltpu.roll(tiles[j], 2 * j, 0) if j else tiles[j]
        w_ref[pl.ds((r0 + LANES * j) // 2, 16), cols] = t


def _transpose8(tiles):
    sub = lax.broadcasted_iota(jnp.int32, tiles[0].shape, 0)
    for s in (4, 2, 1):
        m = (sub & s) == 0
        new = list(tiles)
        for g in range(8):
            if g & s:
                continue
            x, y = tiles[g], tiles[g | s]
            new[g] = jnp.where(m, x, pltpu.roll(y, s, 0))
            new[g | s] = jnp.where(m, pltpu.roll(x, 8 - s, 0), y)
        tiles = new
    return tiles


def _load_rows_permuted(x_ref, row0, T):
    blocks = []
    for hi in range(T // 128):
        blocks += _transpose8([_pack(x_ref[pl.ds(row0 + u * (T // 8) + 16 * hi, 16), :]) for u in range(8)])
    return jnp.concatenate(blocks, axis=0)


def _store_rows_unpermuted(x_ref, row0, T, val):
    for hi in range(T // 128):
        tiles = _transpose8([_pack(val[128 * hi + 16 * t:128 * hi + 16 * (t + 1), :]) for t in range(8)])
        for u in range(8):
            x_ref[pl.ds(row0 + u * (T // 8) + 16 * hi, 16), :] = _unpack(tiles[u])


def _store_kv(val, kv_s, halo_s, T):
    first = lax.broadcasted_iota(jnp.int32, (8, LANES), 0) < 2
    for g in range(G):
        col = val[:, LANES * g:LANES * (g + 1)]
        kv_s[g, pl.ds(EXT, T), :] = col
        for e in range(W - 1):
            r = T - EXT + 16 * e
            lo = pltpu.roll(col[r:r + 8], 2, 0)
            hi = pltpu.roll(col[r + 8:r + 16], 2, 0)
            kv_s[g, pl.ds(16 * e, 8), :] = jnp.where(first, halo_s[g, pl.ds(8 * e, 8), :], lo)
            kv_s[g, pl.ds(16 * e + 8, 8), :] = jnp.where(first, lo, hi)
            halo_s[g, pl.ds(8 * e, 8), :] = hi


def _attn_probs(q_s, k_s, i, invalid):
    R = 16
    r0 = R * i
    lane = lax.broadcasted_iota(jnp.int32, (R, LANES), 1)
    m1 = (lane & 1) == 0
    m2 = (lane & 2) == 0
    q = [q_s[g, pl.ds(r0, R), :] for g in range(G)]
    logits = []
    for w in range(W):
        off = EXT + r0 - R * w
        acc = q[0] * k_s[0, pl.ds(off, R), :]
        for g in range(1, G):
            acc = acc + q[g] * k_s[g, pl.ds(off, R), :]
        acc = acc + jnp.where(m1, pltpu.roll(acc, LANES - 1, 1), pltpu.roll(acc, 1, 1))
        acc = acc + jnp.where(m2, pltpu.roll(acc, LANES - 2, 1), pltpu.roll(acc, 2, 1))
        if i < w:
            acc = jnp.where(invalid, -1e9, acc)
        logits.append(acc)
    mx = logits[0]
    for w in range(1, W):
        mx = jnp.maximum(mx, logits[w])
    p = [jnp.exp2(l - mx) for l in logits]
    den = p[0]
    for w in range(1, W):
        den = den + p[w]
    return p, 1.0 / den


def _attn_values(p, inv, v_s, o_s, i):
    R = 16
    r0 = R * i
    for g in range(G):
        acc = p[0] * v_s[g, pl.ds(EXT + r0, R), :]
        for w in range(1, W):
            acc = acc + p[w] * v_s[g, pl.ds(EXT + r0 - R * w, R), :]
        o_s[pl.ds(r0 // 2, R // 2), pl.ds(LANES * g, LANES)] = _pack(acc * inv)


def _kernel(x_hbm, wqkv_hbm, wo_hbm, w1_hbm, b1_ref, w2_hbm, b2_ref, out_hbm,
            wqkv_r, wo_r, wa_s, w1_s, w2_s, xio_s, xp_s, x1_s, xm_s, xn_s, q_s, k_s, v_s, hk_s, hv_s, o_s,
            wsem, xsem, osem, *, T, FC, LAG, ORDER, O_HEAD, TLOOP, KCH, PRB, STAGE):
    S, D = xio_s.shape
    F = w1_s.shape[1]
    NT = S // T
    NC = F // FC
    qscale = (D // H) ** -0.5 * math.log2(math.e)

    RC = D // KCH

    def cp_qkv(p, c):
        r = pl.ds(pl.multiple_of(c * RC, RC), RC)
        cols = pl.ds(pl.multiple_of(p * D, D), D)
        return pltpu.make_async_copy(wqkv_hbm.at[r, cols], wqkv_r.at[p, r], wsem.at[3 + p * KCH + c])

    def perm_cols(p0, p1):
        def body(t, carry):
            p, c = t // KCH, t % KCH
            cp_qkv(p, c).wait()
            for rr in range(0, RC, PRB):
                _permute_cols_block(wqkv_r.at[p], wa_s.at[p], c * (RC // 2) + rr // 2, PRB // 2)
            return carry

        lax.fori_loop(p0 * KCH, p1 * KCH, body, 0)

    def perm_rows():
        def body(n, carry):
            for a in range(4):
                _permute_rows_block(wo_r, wa_s.at[3], 32 * a, n)
            return carry

        cp_wo.wait()
        lax.fori_loop(0, G, body, 0)

    cp_wo = pltpu.make_async_copy(wo_hbm, wo_r, wsem.at[0])
    cp_w1 = pltpu.make_async_copy(w1_hbm, w1_s, wsem.at[1])
    cp_w2 = pltpu.make_async_copy(w2_hbm, w2_s, wsem.at[2])

    def rows(t):
        return pl.ds(pl.multiple_of(t * T, T), T)

    def cp_x(t):
        return pltpu.make_async_copy(x_hbm.at[rows(t)], xio_s.at[rows(t)], xsem.at[t])

    def cp_out(t):
        return pltpu.make_async_copy(xio_s.at[rows(t)], out_hbm.at[rows(t)], osem.at[t])

    def dot(a, b):
        return jnp.dot(a, b, preferred_element_type=F32)

    def wcat(p):
        return _unpack(wa_s[p])

    def xperm(n):
        xp = _load_rows_permuted(xio_s, pl.multiple_of((n % NT) * T, T), T)
        xp_s[n % 2] = xp
        toks = []
        for hi in range(T // 128):
            for g in range(G):
                t = xp[64 * hi:64 * (hi + 1), LANES * g:LANES * (g + 1)]
                toks.append(pltpu.bitcast(t[0:16] | t[16:32] | t[32:48] | t[48:64], F32))
        return toks

    def tie(x, never, tok):
        if tok is None:
            return x
        x0 = jnp.where(never, tok, x[:, :LANES])
        return x0 if x.shape[1] == LANES else jnp.concatenate([x0, x[:, LANES:]], axis=1)

    def ln1(n, never=None, toks=None):
        for i in range(T // 16):
            r = pl.ds(8 * i, 8)
            x = tie(_unpack(xp_s[n % 2, r, :]).astype(F32), never, toks and toks[i])
            x1_s[r, :] = _pack(_layernorm(x))

    def ln2(n, never=None, toks=None):
        s = n % (LAG + 1)
        for i in range(T // 16):
            x = tie(xm_s[s, pl.ds(16 * i, 16), :], never, toks and toks[i])
            xn_s[s, pl.ds(8 * i, 8), :] = _pack(_layernorm(x))

    def step(na, nf, order):
        st = {}
        if na is not None:
            ta = na % NT
            sa = na % (LAG + 1)
            never = lax.broadcasted_iota(jnp.int32, (16, LANES), 0) < jnp.minimum(na, 0)
        if nf is not None:
            tf = nf % NT
            sf = nf % (LAG + 1)

        def tokens(op, count=T // 16):
            if ":" not in op:
                return None
            cols = []
            for src in op.split(":")[1].split("+"):
                if src not in st:
                    return None
                cols += [(st[src], j) for j in range(st[src].shape[1] // LANES)]
            nb = T // 16
            out = []
            for i in range(count):
                pos = i * len(cols) * nb // count
                val, j = cols[pos // nb]
                r = 16 * (pos % nb)
                out.append(val[r:r + 16, LANES * j:LANES * (j + 1)])
            return out

        def pull(val, spec):
            if spec is None or spec.split(".")[0] not in st:
                return val
            name, a, b = spec.split(".")
            toks = st[name][int(a):int(b)]
            nc, nb = val.shape[1] // LANES, T // 16
            at = {divmod((2 * i + 1) * nc * nb // (2 * len(toks)), nb): t for i, t in enumerate(toks)}
            cols = []
            for j in range(nc):
                col = val[:, LANES * j:LANES * (j + 1)]
                if any(jj == j for jj, _ in at):
                    col = jnp.concatenate([tie(col[16 * r:16 * (r + 1)], never, at.get((j, r)))
                                           for r in range(nb)], axis=0)
                cols.append(col)
            return jnp.concatenate(cols, axis=1)

        for op in order:
            op, *specs = op.split("/")
            specs = dict(sp.split("<") for sp in specs)
            if op[0] == "f":
                if nf is None:
                    continue
            elif na is None:
                continue
            if op == "late":
                @pl.when(na == 0)
                def _():
                    perm_cols(2, 3)
                    perm_rows()
            elif op == "xwait":
                cp_x(na + 1).wait()
            elif op == "xp":
                st["xp"] = xperm(na + 1)
            elif op.startswith("ln1"):
                ln1(na + 1, never, tokens(op))
            elif op == "q":
                st["q"] = pull(dot(_unpack(x1_s[...]), wcat(0)), specs.get("y"))
                q = st["q"] * qscale
                for g in range(G):
                    q_s[g] = q[:, LANES * g:LANES * (g + 1)]
            elif op == "k":
                st["k"] = pull(dot(_unpack(x1_s[...]), wcat(1)), specs.get("y"))
                _store_kv(st["k"], k_s, hk_s, T)
            elif op == "v":
                st["v"] = pull(dot(_unpack(x1_s[...]), wcat(2)), specs.get("y"))
                _store_kv(st["v"], v_s, hv_s, T)
            elif op == "qk":
                row = lax.broadcasted_iota(jnp.int32, (16, LANES), 0)
                invalid = row < jnp.where(ta == 0, 2, 0)
                st["p"] = [_attn_probs(q_s, k_s, i, invalid) for i in range(T // 16)]
                st["sm"] = [inv for _, inv in st["p"]]
            elif op == "pv":
                for i in range(T // 16):
                    _attn_values(*st["p"][i], v_s, o_s, i)
            elif op == "wo":
                st["wo"] = _unpack(xp_s[na % 2]).astype(F32) + pull(dot(_unpack(o_s[...]), wcat(3)), specs.get("y"))
                xm_s[sa] = st["wo"]
            elif op.startswith("ln2"):
                ln2(na + LAG, never, tokens(op))
            elif op == "fbeg":
                st["fxn"] = _unpack(xn_s[sf])
                st["facc"] = xm_s[sf] + b2_ref[...].astype(F32)
            elif op == "fend":
                _store_rows_unpermuted(xio_s, pl.multiple_of(tf * T, T), T, st["facc"])
            else:
                c = int(op[1:])
                h = st[f"h{c}"] = pull(dot(st["fxn"], w1_s[:, pl.ds(c * FC, FC)]), specs.get("h"))
                h = _gelu(h + b1_ref[:, pl.ds(c * FC, FC)].astype(F32)).astype(BF16)
                st[f"y{c}"] = pull(dot(h, w2_s[pl.ds(c * FC, FC), :]), specs.get("y"))
                st[f"z{c}"] = st["facc"] = st["facc"] + st[f"y{c}"]

    order = ORDER.split(",")
    assert sorted(int(o[1]) for o in order if o[0] == "f" and o[1].isdigit()) == list(range(NC))

    def start_rest(stage):
        if stage == STAGE[0]:
            for c in range(KCH):
                cp_qkv(2, c).start()
            cp_wo.start()
            cp_x(1).start()
        if stage == STAGE[1]:
            for t in range(2, LAG + 2):
                cp_x(t).start()
            cp_w1.start()
            cp_w2.start()
            for t in range(LAG + 2, NT):
                cp_x(t).start()

    cp_x(0).start()
    for p in range(2):
        for c in range(KCH):
            cp_qkv(p, c).start()
    start_rest(0)
    hk_s[...] = jnp.zeros(hk_s.shape, F32)
    hv_s[...] = jnp.zeros(hv_s.shape, F32)
    cp_x(0).wait()
    xperm(0)

    def ln_first(i, carry):
        r = pl.ds(pl.multiple_of(i * 32, 32), 32)
        x1_s[r, :] = _pack(_layernorm(_unpack(xp_s[0, r, :]).astype(F32)))
        xm_s[LAG, pl.ds(pl.multiple_of(i * 64, 64), 64), :] = jnp.zeros((64, D), F32)
        return carry

    lax.fori_loop(0, T // 64, ln_first, 0)
    start_rest(1)

    if "late" in O_HEAD:
        perm_cols(0, 2)
    else:
        perm_cols(0, 3)
        perm_rows()

    start_rest(2)

    def head(n, carry):
        step(n, None, O_HEAD.split(","))
        return carry

    lax.fori_loop(0, LAG, head, 0)
    cp_w1.wait()
    cp_w2.wait()

    def steady(n, carry):
        @pl.when(n + 1 < NT)
        def _():
            cp_x(n + 1).wait()

        step(n, n - LAG, order)

        @pl.when(n - LAG >= NT)
        def _():
            cp_out(n - LAG - NT).start()

        return carry

    lax.fori_loop(LAG, 2 * NT, steady, 0)
    ln2(2 * NT - 1)

    def tail(n, carry):
        if TLOOP:
            sf = n % (LAG + 1)

            def chunk(c, carry):
                c0 = pl.multiple_of(c * FC, FC)
                h = dot(_unpack(xn_s[sf]), w1_s[:, pl.ds(c0, FC)])
                h = _gelu(h + b1_ref[:, pl.ds(c0, FC)].astype(F32)).astype(BF16)
                xm_s[sf] += dot(h, w2_s[pl.ds(c0, FC), :])
                return carry

            lax.fori_loop(0, NC, chunk, 0)
            step(None, n, ["fbeg", "fend"])
        else:
            step(None, n, order)
        cp_out(n - NT).start()
        return carry

    lax.fori_loop(2 * NT - LAG, 2 * NT, tail, 0)
    for t in range(NT):
        cp_out(t).wait()


def _forward(A_x, A_wqkv, A_wo, B_w1, B_b1, B_w2, B_b2, T=256, FC=512, LAG=3, TLOOP=True, KCH=4, PRB=32, STAGE=(0, 0),
             ORDER="fbeg,xp,k/y<xp.0.16,q,qk,f0,f1/h<sm.0.8/y<sm.8.16,v,pv,f2,f3,ln2:y2+y3,f4,f5,ln1:y4+y5,f6,fend,wo",
             O_HEAD="k,ln2:k,q,late,xwait,xp,qk,v,pv,wo,ln1"):
    B, S, D = A_x.shape
    F = B_w1.shape[1]
    assert B == 1 and D == G * LANES and S % T == 0 and F % FC == 0 and T % 128 == 0 and 2 <= LAG < S // T
    any_spec = pl.BlockSpec(memory_space=pl.ANY)
    vmem_spec = pl.BlockSpec(memory_space=pltpu.VMEM)
    out = pl.pallas_call(
        functools.partial(_kernel, T=T, FC=FC, LAG=LAG, ORDER=ORDER, O_HEAD=O_HEAD, TLOOP=TLOOP, KCH=KCH, PRB=PRB, STAGE=STAGE),
        in_specs=[any_spec, any_spec, any_spec, any_spec, vmem_spec, any_spec, vmem_spec],
        out_specs=any_spec,
        out_shape=jax.ShapeDtypeStruct((S, D), A_x.dtype),
        scratch_shapes=[
            pltpu.VMEM((3, D, D), BF16),
            pltpu.VMEM((D, D), BF16),
            pltpu.VMEM((4, D // 2, D), U32),
            pltpu.VMEM((D, F), BF16),
            pltpu.VMEM((F, D), BF16),
            pltpu.VMEM((S, D), BF16),
            pltpu.VMEM((2, T // 2, D), U32),
            pltpu.VMEM((T // 2, D), U32),
            pltpu.VMEM((LAG + 1, T, D), F32),
            pltpu.VMEM((LAG + 1, T // 2, D), U32),
            pltpu.VMEM((G, T, LANES), F32),
            pltpu.VMEM((G, T + EXT, LANES), F32),
            pltpu.VMEM((G, T + EXT, LANES), F32),
            pltpu.VMEM((G, EXT // 2, LANES), F32),
            pltpu.VMEM((G, EXT // 2, LANES), F32),
            pltpu.VMEM((T // 2, D), U32),
            pltpu.SemaphoreType.DMA((3 + 3 * KCH,)),
            pltpu.SemaphoreType.DMA((S // T,)),
            pltpu.SemaphoreType.DMA((S // T,)),
        ],
        compiler_params=pltpu.CompilerParams(vmem_limit_bytes=100 * 1024 * 1024),
    )(A_x.reshape(S, D), A_wqkv, A_wo, B_w1, B_b1.reshape(1, F), B_w2, B_b2.reshape(1, D))
    return out.reshape(B, S, D)


@jax.jit
def pallas_interleave_layers__sliding_local_dilated__dense_activation_gelu__prompt_kernel(
    A_x: jax.Array,
    A_wqkv: jax.Array,
    A_wo: jax.Array,
    B_x: jax.Array,
    B_w1: jax.Array,
    B_b1: jax.Array,
    B_w2: jax.Array,
    B_b2: jax.Array,
):
    del B_x
    return _forward(A_x, A_wqkv, A_wo, B_w1, B_b1, B_w2, B_b2)
```

```python
import functools
import math

import jax
import jax.numpy as jnp
from jax import lax
import jax.experimental.pallas as pl
import jax.experimental.pallas.tpu as pltpu

H = 32
W = 8
LANES = 128
G = 8
EXT = 16 * (W - 1)
EPS = 1e-5
F32 = jnp.float32
BF16 = jnp.bfloat16
U32 = jnp.uint32


def _layernorm(x):
    m = jnp.mean(x, axis=-1, keepdims=True)
    xc = x - m
    v = jnp.mean(xc * xc, axis=-1, keepdims=True)
    return xc * lax.rsqrt(v + EPS)


def _gelu(x):
    c = math.sqrt(2.0 / math.pi)
    hx = 0.5 * x
    return hx + hx * jnp.tanh(x * (c + (c * 0.044715) * (x * x)))


def _pack(x):
    return pltpu.bitcast(x.astype(BF16), U32)


def _unpack(u):
    return pltpu.bitcast(u, BF16)


def _barrel(tiles, b):
    for t in (1, 2, 4):
        m = (b & t) != 0
        tiles = [jnp.where(m, tiles[(j + t) % 8], tiles[j]) for j in range(8)]
    return tiles


def _permute_cols_block(src_ref, w_ref, h0, hb, hint=lambda t: t):
    rows = pl.ds(pl.multiple_of(2 * h0, 2 * hb), 2 * hb)
    tiles = [_pack(src_ref[rows, pl.ds(LANES * g, LANES)]) for g in range(G)]
    tiles[0] = hint(tiles[0])
    b = (lax.broadcasted_iota(jnp.int32, tiles[0].shape, 1) >> 2) & 7
    tiles = _barrel(tiles, b)
    for j in range(G):
        t = tiles[j]
        if j:
            t = jnp.where(b >= j, pltpu.roll(t, 4 * j, 1), pltpu.roll(t, LANES - 32 + 4 * j, 1))
        w_ref[pl.ds(pl.multiple_of(h0, hb), hb), pl.ds(LANES * j, LANES)] = t


def _permute_rows_block(src_ref, w_ref, r0, n, hint=lambda t: t):
    cols = pl.ds(pl.multiple_of(n * LANES, LANES), LANES)
    tiles = [_pack(src_ref[pl.ds(r0 + LANES * g, 32), cols]) for g in range(G)]
    tiles[0] = hint(tiles[0])
    b = lax.broadcasted_iota(jnp.int32, tiles[0].shape, 0) >> 1
    tiles = _barrel(tiles, b)
    for j in range(G):
        t = pltpu.roll(tiles[j], 2 * j, 0) if j else tiles[j]
        w_ref[pl.ds((r0 + LANES * j) // 2, 16), cols] = t


def _transpose8(tiles):
    sub = lax.broadcasted_iota(jnp.int32, tiles[0].shape, 0)
    for s in (4, 2, 1):
        m = (sub & s) == 0
        new = list(tiles)
        for g in range(8):
            if g & s:
                continue
            x, y = tiles[g], tiles[g | s]
            new[g] = jnp.where(m, x, pltpu.roll(y, s, 0))
            new[g | s] = jnp.where(m, pltpu.roll(x, 8 - s, 0), y)
        tiles = new
    return tiles


def _load_rows_permuted(x_ref, row0, T):
    blocks = []
    for hi in range(T // 128):
        blocks += _transpose8([_pack(x_ref[pl.ds(row0 + u * (T // 8) + 16 * hi, 16), :]) for u in range(8)])
    return jnp.concatenate(blocks, axis=0)


def _store_rows_unpermuted(x_ref, row0, T, cols, val):
    for hi in range(T // 128):
        tiles = _transpose8([_pack(val[128 * hi + 16 * t:128 * hi + 16 * (t + 1), :]) for t in range(8)])
        for u in range(8):
            x_ref[pl.ds(row0 + u * (T // 8) + 16 * hi, 16), cols] = _unpack(tiles[u])


def _store_kv(val, kv_s, halo_s, T):
    first = lax.broadcasted_iota(jnp.int32, (8, LANES), 0) < 2
    for g in range(G):
        col = val[:, LANES * g:LANES * (g + 1)]
        kv_s[g, pl.ds(EXT, T), :] = col
        for e in range(W - 1):
            r = T - EXT + 16 * e
            lo = pltpu.roll(col[r:r + 8], 2, 0)
            hi = pltpu.roll(col[r + 8:r + 16], 2, 0)
            kv_s[g, pl.ds(16 * e, 8), :] = jnp.where(first, halo_s[g, pl.ds(8 * e, 8), :], lo)
            kv_s[g, pl.ds(16 * e + 8, 8), :] = jnp.where(first, lo, hi)
            halo_s[g, pl.ds(8 * e, 8), :] = hi


def _attn_probs(q_s, k_s, i, invalid):
    R = 16
    r0 = R * i
    lane = lax.broadcasted_iota(jnp.int32, (R, LANES), 1)
    m1 = (lane & 1) == 0
    m2 = (lane & 2) == 0
    q = [q_s[g, pl.ds(r0, R), :] for g in range(G)]
    logits = []
    for w in range(W):
        off = EXT + r0 - R * w
        acc = q[0] * k_s[0, pl.ds(off, R), :]
        for g in range(1, G):
            acc = acc + q[g] * k_s[g, pl.ds(off, R), :]
        acc = acc + jnp.where(m1, pltpu.roll(acc, LANES - 1, 1), pltpu.roll(acc, 1, 1))
        acc = acc + jnp.where(m2, pltpu.roll(acc, LANES - 2, 1), pltpu.roll(acc, 2, 1))
        if i < w:
            acc = jnp.where(invalid, -1e9, acc)
        logits.append(acc)
    mx = logits[0]
    for w in range(1, W):
        mx = jnp.maximum(mx, logits[w])
    p = [jnp.exp2(l - mx) for l in logits]
    den = p[0]
    for w in range(1, W):
        den = den + p[w]
    return p, 1.0 / den


def _attn_values(p, inv, v_s, o_s, i):
    R = 16
    r0 = R * i
    for g in range(G):
        acc = p[0] * v_s[g, pl.ds(EXT + r0, R), :]
        for w in range(1, W):
            acc = acc + p[w] * v_s[g, pl.ds(EXT + r0 - R * w, R), :]
        o_s[pl.ds(r0 // 2, R // 2), pl.ds(LANES * g, LANES)] = _pack(acc * inv)


def _kernel(x_hbm, wqkv_hbm, wo_hbm, w1_hbm, b1_in, w2_hbm, b2_in, out_hbm,
            wqkv_r, wo_r, wq_s, wk_s, wv_s, wo_s, qh_s, kh_s, w1_s, w2_s, xio_s, xp_s, x1_s, xm_s, xn_s, q_s, k_s, v_s, hk_s, hv_s, o_s,
            b1_ref, b2_ref,
            wsem, xsem, osem, *, T, FC, LAG, ORDER, O_A, O_B, O_C, TFIN, KCH, PRB, TLN, PFREE, DS, DUN, XW):
    S, D = xio_s.shape
    F = w1_s.shape[1]
    NT = S // T
    NC = F // FC
    qscale = (D // H) ** -0.5 * math.log2(math.e)

    RC = D // KCH

    def cp_qkv(p, c):
        r = pl.ds(pl.multiple_of(c * RC, RC), RC)
        cols = pl.ds(pl.multiple_of(p * D, D), D)
        return pltpu.make_async_copy(wqkv_hbm.at[r, cols], wqkv_r.at[p, r], wsem.at[3 + p * KCH + c])

    cp_wo = pltpu.make_async_copy(wo_hbm, wo_r, wsem.at[0])
    cp_w1 = pltpu.make_async_copy(w1_hbm, w1_s, wsem.at[1])
    cp_w2 = pltpu.make_async_copy(w2_hbm, w2_s, wsem.at[2])

    def rows(t):
        return pl.ds(pl.multiple_of(t * T, T), T)

    def cp_x(t):
        return pltpu.make_async_copy(x_hbm.at[rows(t)], xio_s.at[rows(t)], xsem.at[t])

    def cp_out(t):
        return pltpu.make_async_copy(xio_s.at[rows(t)], out_hbm.at[rows(t)], osem.at[t])

    def dot(a, b):
        return jnp.dot(a, b, preferred_element_type=F32)

    def xperm(n):
        xp = _load_rows_permuted(xio_s, pl.multiple_of((n % NT) * T, T), T)
        xp_s[n % (LAG + 1)] = xp
        toks = []
        for hi in range(T // 128):
            for g in range(G):
                t = xp[64 * hi:64 * (hi + 1), LANES * g:LANES * (g + 1)]
                toks.append(pltpu.bitcast(t[0:16] | t[16:32] | t[32:48] | t[48:64], F32))
        return toks

    def tie(x, never, tok):
        if tok is None:
            return x
        x0 = jnp.where(never, tok, x[:, :LANES])
        return x0 if x.shape[1] == LANES else jnp.concatenate([x0, x[:, LANES:]], axis=1)

    def ln1(n, x1, never, toks, a, b):
        out = []
        for i in range(a, b):
            r = pl.ds(8 * i, 8)
            x = tie(_unpack(xp_s[n % (LAG + 1), r, :]).astype(F32), never, toks and toks[i - a])
            y = _layernorm(x)
            x1[r, :] = _pack(y)
            out.append(y[:, D - LANES:])
        return out

    def ln2(n, never, toks, a, b):
        s = n % (LAG + 1)
        out = []
        for i in range(a, b):
            x = tie(xm_s[s, pl.ds(16 * i, 16), :], never, toks and toks[i - a])
            y = _layernorm(x)
            xn_s[s, pl.ds(8 * i, 8), :] = _pack(y)
            out.append(y[:, D - LANES:])
        return out

    def step(na, nf, order, head=False):
        st = {}
        if na is not None:
            ta = na % NT
            sa = na % (LAG + 1)
            never = lax.broadcasted_iota(jnp.int32, (16, LANES), 0) < jnp.minimum(na, 0)
            x1, x1n = (x1_s.at[na], o_s) if head else (x1_s.at[LAG], x1_s.at[LAG])
            qr, kr = (qh_s.at[na], kh_s.at[na]) if head else (q_s, k_s)
        if nf is not None:
            tf = nf % NT
            sf = nf % (LAG + 1)

        def tokens(op, count=T // 16):
            if ":" not in op:
                return None
            cols = []
            op, *pad = op.split("~")
            skip, lead = map(int, pad) if pad else (0, 0)
            for src in op.split(":")[1].split("+"):
                if src not in st:
                    return None
                cols += [(st[src], j) for j in range(st[src].shape[1] // LANES)]
            nb = T // 16
            out = []
            for i in range(count):
                pos = (i + skip) * len(cols) * nb // (count + skip + lead)
                val, j = cols[pos // nb]
                r = 16 * (pos % nb)
                out.append(val[r:r + 16, LANES * j:LANES * (j + 1)])
            return out

        def pull(val, spec):
            if spec is None or spec.split(".")[0] not in st:
                return val
            name, a, b = spec.split(".")
            toks = st[name][int(a):int(b)]
            nc, nb = val.shape[1] // LANES, T // 16
            at = {divmod((2 * i + 1) * nc * nb // (2 * len(toks)), nb): t for i, t in enumerate(toks)}
            cols = []
            for j in range(nc):
                col = val[:, LANES * j:LANES * (j + 1)]
                if any(jj == j for jj, _ in at):
                    col = jnp.concatenate([tie(col[16 * r:16 * (r + 1)], never, at.get((j, r)))
                                           for r in range(nb)], axis=0)
                cols.append(col)
            return jnp.concatenate(cols, axis=1)

        for op in order:
            op, *specs = op.split("/")
            specs = dict(sp.split("<") for sp in specs)
            if op[0] == "f":
                if nf is None:
                    continue
            elif na is None:
                continue
            if op.startswith("ln"):
                a, b = map(int, op.split(":")[0].split("@")[1:] or (0, T // 16))
            if op.startswith("perm"):
                if op.startswith("permq"):
                    h0 = jnp.maximum(na - 1, 0) * (D // 4)
                    jobs = [(_permute_cols_block, wqkv_r.at[jnp.where(na == 0, 1, 0)], wq_s, h0 + 16 * i, 16)
                            for i in range(D // 64)]
                else:
                    nv, no = -(-D // 32 // LAG), -(-G // LAG)
                    h0 = jnp.minimum(na * nv, D // 32 - nv) * 16
                    n0 = jnp.minimum(na * no, G - no)
                    jv = [(_permute_cols_block, wqkv_r.at[2], wv_s, h0 + 16 * i, 16) for i in range(nv)]
                    jo = [(_permute_rows_block, wo_r, wo_s, 32 * (i % 4), n0 + i // 4) for i in range(4 * no)]
                    jobs = [j for pair in zip(jv + [None] * len(jo), jo) for j in pair if j] + jv[len(jo):]
                toks = [None] * PFREE + tokens(op, len(jobs) - PFREE)
                for (fn, *args), tok in zip(jobs, toks):
                    tok = None if tok is None else pltpu.bitcast(tok, U32)
                    fn(*args, hint=functools.partial(tie, never=never, tok=tok))
            elif op == "x1":
                x1[...] = o_s[...]
            elif op == "xp":
                st["xp"] = xperm(na + 1)
            elif op.startswith("ln1"):
                st["l1"] = ln1(na + 1, x1n, never, tokens(op, b - a), a, b)
            elif op == "q":
                st["q"] = pull(dot(_unpack(x1[...]), _unpack(wq_s[...])), specs.get("y"))
                q = st["q"] * qscale
                for g in range(G):
                    qr[g] = q[:, LANES * g:LANES * (g + 1)]
            elif op == "k":
                st["k"] = pull(dot(_unpack(x1[...]), _unpack(wk_s[...])), specs.get("y"))
                _store_kv(st["k"], kr, hk_s, T)
            elif op == "v":
                st["v"] = pull(dot(_unpack(x1[...]), _unpack(wv_s[...])), specs.get("y"))
                _store_kv(st["v"], v_s, hv_s, T)
            elif op == "qk":
                row = lax.broadcasted_iota(jnp.int32, (16, LANES), 0)
                invalid = row < jnp.where(ta == 0, 2, 0)
                st["p"] = [_attn_probs(qr, kr, i, invalid) for i in range(T // 16)]
                st["sm"] = [inv for _, inv in st["p"]]
            elif op == "pv":
                for i in range(T // 16):
                    _attn_values(*st["p"][i], v_s, o_s, i)
            elif op == "wo":
                st["wo"] = _unpack(xp_s[sa]).astype(F32) + pull(dot(_unpack(o_s[...]), _unpack(wo_s[...])), specs.get("y"))
                xm_s[sa] = st["wo"]
            elif op.startswith("ln2"):
                st["l2"] = ln2(na + LAG, never, tokens(op, b - a), a, b)
            elif op == "fbeg":
                st["fxn"] = _unpack(xn_s[sf])
                st["facc"] = xm_s[sf] + b2_ref[...].astype(F32)
            elif op == "fend":
                _store_rows_unpermuted(xio_s, pl.multiple_of(tf * T, T), T, slice(None), st["facc"])
            else:
                c = int(op[1:])
                h = st[f"h{c}"] = pull(dot(st["fxn"], w1_s[:, pl.ds(c * FC, FC)]), specs.get("h"))
                h = _gelu(h + b1_ref[:, pl.ds(c * FC, FC)].astype(F32)).astype(BF16)
                st[f"y{c}"] = pull(dot(h, w2_s[pl.ds(c * FC, FC), :]), specs.get("y"))
                st[f"z{c}"] = st["facc"] = st["facc"] + st[f"y{c}"]

    order = ORDER.split(",")
    assert sorted(int(o[1]) for o in order if o[0] == "f" and o[1].isdigit()) == list(range(NC))

    assert LAG == 3 and KCH == 4
    fetch = ([cp_x(0)] + [cp_qkv(1, c) for c in range(4)] + [cp_x(1), cp_x(2), cp_qkv(0, 0), cp_qkv(0, 1), cp_x(3),
               cp_qkv(0, 2), cp_qkv(0, 3), cp_wo] + [cp_qkv(2, c) for c in range(4)] + [cp_x(4), cp_w1, cp_w2]
               + [cp_x(t) for t in range(5, NT)])
    for cp in fetch[:DS[0]]:
        cp.start()
    b1_ref[...] = b1_in[...].astype(F32).reshape(1, F)
    b2_ref[...] = b2_in[...].astype(F32).reshape(1, D)
    hk_s[...] = jnp.zeros(hk_s.shape, F32)
    hv_s[...] = jnp.zeros(hv_s.shape, F32)
    cp_x(0).wait()
    xperm(0)

    def ln_first(i, carry):
        r = pl.ds(pl.multiple_of(i * 32, 32), 32)
        o_s[r, :] = _pack(_layernorm(_unpack(xp_s[0, r, :]).astype(F32)))
        xm_s[LAG, pl.ds(pl.multiple_of(i * 64, 64), 64), :] = jnp.zeros((64, D), F32)
        return carry

    lax.fori_loop(0, T // 64, ln_first, 0)
    for cp in fetch[DS[0]:DS[1]]:
        cp.start()

    def perm_k(c, carry):
        cp_qkv(1, c).wait()
        for rr in range(0, RC, PRB):
            _permute_cols_block(wqkv_r.at[1], wk_s, c * (RC // 2) + rr // 2, PRB // 2)
        return carry

    lax.fori_loop(0, KCH, perm_k, 0)
    for cp in fetch[DS[1]:]:
        cp.start()

    def head_k(n, carry):
        cp_x(n + 1).wait()

        @pl.when(n > 0)
        def _():
            cp_qkv(0, 2 * n - 2).wait()
            cp_qkv(0, 2 * n - 1).wait()

        step(n, None, O_A.split(","), head=True)
        return carry

    def head_q(n, carry):
        cp_qkv(2, n + 1).wait()
        step(n, None, O_B.split(","), head=True)
        return carry

    def head_v(n, carry):
        step(n, None, O_C.split(","), head=True)
        return carry

    lax.fori_loop(0, LAG, head_k, 0)
    x1_s[LAG] = o_s[...]
    cp_wo.wait()
    cp_qkv(2, 0).wait()
    lax.fori_loop(0, LAG, head_q, 0)
    lax.fori_loop(0, LAG, head_v, 0)
    cp_w1.wait()
    cp_w2.wait()

    if XW:
        for t in range(LAG + 1, NT):
            cp_x(t).wait()

    def steady(n, carry):
        if not XW:
            @pl.when(n + 1 < NT)
            def _():
                cp_x(n + 1).wait()

        step(n, n - LAG, order)
        return carry

    lax.fori_loop(LAG, 2 * NT, steady, 0)
    for t in range(NT - LAG):
        cp_out(t).start()
    last = 2 * NT - 1
    CW = D // 4

    def finish(n, j, never, toks):
        for g in range(CW // LANES):
            cols = pl.ds(pl.multiple_of(j * CW + g * LANES, LANES), LANES)
            val = xm_s[n % (LAG + 1), :, cols] + b2_ref[:, cols]
            val = jnp.concatenate([tie(val[16 * r:16 * (r + 1)], never, toks.get((g, r))) for r in range(T // 16)], axis=0)
            _store_rows_unpermuted(xio_s, pl.multiple_of((n % NT) * T, T), T, cols, val)

    def tail(n, carry):
        sf = n % (LAG + 1)
        sl = jnp.where(n < last, last, last + 1) % (LAG + 1)

        def chunk(c, carry):
            c0 = pl.multiple_of(c * FC, FC)
            i = jnp.minimum((n - (2 * NT - LAG)) * NC + c, T // 32 - 1)
            x = xm_s[sl, pl.ds(pl.multiple_of(32 * i, 32), 32), :]
            h = dot(_unpack(xn_s[sf]), w1_s[:, pl.ds(c0, FC)])
            if TFIN:
                never = lax.broadcasted_iota(jnp.int32, (16, LANES), 0) < jnp.minimum(n, 0)
                toks = {}
                for u, (tc, tr) in enumerate(TFIN):
                    for r in range(8):
                        toks[(u // 2, 8 * (u % 2) + r)] = h[tr:tr + 16, LANES * tc:LANES * (tc + 1)]
                finish(jnp.maximum(n - 1, 2 * NT - LAG), jnp.minimum(c, 3), never, toks)
            h = _gelu(h + b1_ref[:, pl.ds(c0, FC)]).astype(BF16)
            y = xm_s[sf] + dot(h, w2_s[pl.ds(c0, FC), :])
            xn = _pack(_layernorm(x))
            xn_s[sl, pl.ds(pl.multiple_of(16 * i, 16), 16), :] = xn
            if TLN is not None:
                tok = xn[:, :LANES]
                for g in range(1, G):
                    tok = tok | xn[:, LANES * g:LANES * (g + 1)]
                a = LANES * TLN
                yc = jnp.concatenate([tie(y[:16, a:a + LANES], never, pltpu.bitcast(tok, F32)), y[16:, a:a + LANES]], axis=0)
                y = jnp.concatenate([y[:, :a], yc, y[:, a + LANES:]], axis=1)
            xm_s[sf] = y
            return carry

        lax.fori_loop(0, NC, chunk, 0)
        if TFIN:
            @pl.when(n > 2 * NT - LAG)
            def _():
                cp_out(n - 1 - NT).start()
        else:
            step(None, n, ["fbeg", "fend"])
            cp_out(n - NT).start()
        return carry

    lax.fori_loop(2 * NT - LAG, 2 * NT, tail, 0)

    def cp_last(j):
        cols = pl.ds(pl.multiple_of(j * CW, CW), CW)
        return pltpu.make_async_copy(xio_s.at[rows(NT - 1), cols], out_hbm.at[rows(NT - 1), cols], osem.at[NT - 1 + j])

    def drain(j, carry):
        finish(last, j, None, {})
        cp_last(j).start()
        return carry

    lax.fori_loop(0, D // CW, drain, 0, unroll=DUN)
    for t in range(NT - 1):
        cp_out(t).wait()
    for j in range(D // CW):
        cp_last(j).wait()


def _forward(A_x, A_wqkv, A_wo, B_w1, B_b1, B_w2, B_b2, T=256, FC=512, LAG=3, TFIN=((0,0),(1,0),(2,0),(3,0)), KCH=4, PRB=32, PFREE=1, XW=0, DUN=True, DS=(6, 13), TLN=2,
             ORDER="fbeg,xp,k/y<xp.0.16,q,qk,f0,f1/h<sm.0.8/y<sm.8.16,v,pv,f2,f3,ln2:y2+y3~0~1,f4,f5,ln1:y4+y5~0~1,f6,wo,fend",
             O_A="x1,xp,k,ln1:k~0~2,permq:k~0~2", O_B="q,permv:q~0~2", O_C="qk,v,ln2:v~48~0,pv,wo"):
    B, S, D = A_x.shape
    F = B_w1.shape[1]
    assert B == 1 and D == G * LANES and S % T == 0 and F % FC == 0 and T % 128 == 0 and 2 <= LAG < S // T
    any_spec = pl.BlockSpec(memory_space=pl.ANY)
    vmem_spec = pl.BlockSpec(memory_space=pltpu.VMEM)
    out = pl.pallas_call(
        functools.partial(_kernel, T=T, FC=FC, LAG=LAG, ORDER=ORDER, O_A=O_A, O_B=O_B, O_C=O_C, TFIN=TFIN, KCH=KCH, PRB=PRB, PFREE=PFREE, XW=XW, DUN=DUN, DS=DS, TLN=TLN),
        in_specs=[any_spec, any_spec, any_spec, any_spec, vmem_spec, any_spec, vmem_spec],
        out_specs=any_spec,
        out_shape=jax.ShapeDtypeStruct((S, D), A_x.dtype),
        scratch_shapes=[
            pltpu.VMEM((3, D, D), BF16),
            pltpu.VMEM((D, D), BF16),
            pltpu.VMEM((D // 2, D), U32),
            pltpu.VMEM((D // 2, D), U32),
            pltpu.VMEM((D // 2, D), U32),
            pltpu.VMEM((D // 2, D), U32),
            pltpu.VMEM((LAG, G, T, LANES), F32),
            pltpu.VMEM((LAG, G, T + EXT, LANES), F32),
            pltpu.VMEM((D, F), BF16),
            pltpu.VMEM((F, D), BF16),
            pltpu.VMEM((S, D), BF16),
            pltpu.VMEM((LAG + 1, T // 2, D), U32),
            pltpu.VMEM((LAG + 1, T // 2, D), U32),
            pltpu.VMEM((LAG + 1, T, D), F32),
            pltpu.VMEM((LAG + 1, T // 2, D), U32),
            pltpu.VMEM((G, T, LANES), F32),
            pltpu.VMEM((G, T + EXT, LANES), F32),
            pltpu.VMEM((G, T + EXT, LANES), F32),
            pltpu.VMEM((G, EXT // 2, LANES), F32),
            pltpu.VMEM((G, EXT // 2, LANES), F32),
            pltpu.VMEM((T // 2, D), U32),
            pltpu.VMEM((1, F), F32),
            pltpu.VMEM((1, D), F32),
            pltpu.SemaphoreType.DMA((3 + 3 * KCH,)),
            pltpu.SemaphoreType.DMA((S // T,)),
            pltpu.SemaphoreType.DMA((S // T + 3,)),
        ],
        compiler_params=pltpu.CompilerParams(vmem_limit_bytes=100 * 1024 * 1024),
    )(A_x.reshape(S, D), A_wqkv, A_wo, B_w1, B_b1, B_w2, B_b2)
    return out.reshape(B, S, D)


@jax.jit
def pallas_interleave_layers__sliding_local_dilated__dense_activation_gelu__prompt_kernel(
    A_x: jax.Array,
    A_wqkv: jax.Array,
    A_wo: jax.Array,
    B_x: jax.Array,
    B_w1: jax.Array,
    B_b1: jax.Array,
    B_w2: jax.Array,
    B_b2: jax.Array,
):
    del B_x
    return _forward(A_x, A_wqkv, A_wo, B_w1, B_b1, B_w2, B_b2)
```

```python
import functools
import math

import jax
import jax.numpy as jnp
from jax import lax
import jax.experimental.pallas as pl
import jax.experimental.pallas.tpu as pltpu

H = 32
W = 8
LANES = 128
G = 8
EXT = 16 * (W - 1)
EPS = 1e-5
F32 = jnp.float32
BF16 = jnp.bfloat16
U32 = jnp.uint32


def _layernorm(x):
    m = jnp.mean(x, axis=-1, keepdims=True)
    xc = x - m
    v = jnp.mean(xc * xc, axis=-1, keepdims=True)
    return xc * lax.rsqrt(v + EPS)


def _gelu(x):
    c = math.sqrt(2.0 / math.pi)
    hx = 0.5 * x
    return hx + hx * jnp.tanh(x * (c + (c * 0.044715) * (x * x)))


def _pack(x):
    return pltpu.bitcast(x.astype(BF16), U32)


def _unpack(u):
    return pltpu.bitcast(u, BF16)


def _barrel(tiles, b):
    for t in (1, 2, 4):
        m = (b & t) != 0
        tiles = [jnp.where(m, tiles[(j + t) % 8], tiles[j]) for j in range(8)]
    return tiles


def _permute_cols_block(src_ref, w_ref, h0, hb, hint=lambda t: t):
    rows = pl.ds(pl.multiple_of(2 * h0, 2 * hb), 2 * hb)
    tiles = [_pack(src_ref[rows, pl.ds(LANES * g, LANES)]) for g in range(G)]
    tiles[0] = hint(tiles[0])
    b = (lax.broadcasted_iota(jnp.int32, tiles[0].shape, 1) >> 2) & 7
    tiles = _barrel(tiles, b)
    for j in range(G):
        t = tiles[j]
        if j:
            t = jnp.where(b >= j, pltpu.roll(t, 4 * j, 1), pltpu.roll(t, LANES - 32 + 4 * j, 1))
        w_ref[pl.ds(pl.multiple_of(h0, hb), hb), pl.ds(LANES * j, LANES)] = t


def _permute_rows_block(src_ref, w_ref, r0, n, hint=lambda t: t):
    cols = pl.ds(pl.multiple_of(n * LANES, LANES), LANES)
    tiles = [_pack(src_ref[pl.ds(r0 + LANES * g, 32), cols]) for g in range(G)]
    tiles[0] = hint(tiles[0])
    b = lax.broadcasted_iota(jnp.int32, tiles[0].shape, 0) >> 1
    tiles = _barrel(tiles, b)
    for j in range(G):
        t = pltpu.roll(tiles[j], 2 * j, 0) if j else tiles[j]
        w_ref[pl.ds((r0 + LANES * j) // 2, 16), cols] = t


def _transpose8(tiles):
    sub = lax.broadcasted_iota(jnp.int32, tiles[0].shape, 0)
    for s in (4, 2, 1):
        m = (sub & s) == 0
        new = list(tiles)
        for g in range(8):
            if g & s:
                continue
            x, y = tiles[g], tiles[g | s]
            new[g] = jnp.where(m, x, pltpu.roll(y, s, 0))
            new[g | s] = jnp.where(m, pltpu.roll(x, 8 - s, 0), y)
        tiles = new
    return tiles


def _load_rows_permuted(x_ref, row0, T):
    blocks = []
    for hi in range(T // 128):
        blocks += _transpose8([_pack(x_ref[pl.ds(row0 + u * (T // 8) + 16 * hi, 16), :]) for u in range(8)])
    return jnp.concatenate(blocks, axis=0)


def _store_rows_unpermuted(x_ref, row0, T, cols, val):
    for hi in range(T // 128):
        tiles = _transpose8([_pack(val[128 * hi + 16 * t:128 * hi + 16 * (t + 1), :]) for t in range(8)])
        for u in range(8):
            x_ref[pl.ds(row0 + u * (T // 8) + 16 * hi, 16), cols] = _unpack(tiles[u])


def _store_kv(val, kv_s, halo_s, T):
    first = lax.broadcasted_iota(jnp.int32, (8, LANES), 0) < 2
    for g in range(G):
        col = val[:, LANES * g:LANES * (g + 1)]
        kv_s[g, pl.ds(EXT, T), :] = col
        for e in range(W - 1):
            r = T - EXT + 16 * e
            lo = pltpu.roll(col[r:r + 8], 2, 0)
            hi = pltpu.roll(col[r + 8:r + 16], 2, 0)
            kv_s[g, pl.ds(16 * e, 8), :] = jnp.where(first, halo_s[g, pl.ds(8 * e, 8), :], lo)
            kv_s[g, pl.ds(16 * e + 8, 8), :] = jnp.where(first, lo, hi)
            halo_s[g, pl.ds(8 * e, 8), :] = hi


def _attn_probs(q_s, k_s, i, invalid):
    R = 16
    r0 = R * i
    lane = lax.broadcasted_iota(jnp.int32, (R, LANES), 1)
    m1 = (lane & 1) == 0
    m2 = (lane & 2) == 0
    q = [q_s[g, pl.ds(r0, R), :] for g in range(G)]
    logits = []
    for w in range(W):
        off = EXT + r0 - R * w
        acc = q[0] * k_s[0, pl.ds(off, R), :]
        for g in range(1, G):
            acc = acc + q[g] * k_s[g, pl.ds(off, R), :]
        acc = acc + jnp.where(m1, pltpu.roll(acc, LANES - 1, 1), pltpu.roll(acc, 1, 1))
        acc = acc + jnp.where(m2, pltpu.roll(acc, LANES - 2, 1), pltpu.roll(acc, 2, 1))
        if i < w:
            acc = jnp.where(invalid, -1e9, acc)
        logits.append(acc)
    mx = logits[0]
    for w in range(1, W):
        mx = jnp.maximum(mx, logits[w])
    p = [jnp.exp2(l - mx) for l in logits]
    den = p[0]
    for w in range(1, W):
        den = den + p[w]
    return p, 1.0 / den


def _attn_values(p, inv, v_s, o_s, i):
    R = 16
    r0 = R * i
    for g in range(G):
        acc = p[0] * v_s[g, pl.ds(EXT + r0, R), :]
        for w in range(1, W):
            acc = acc + p[w] * v_s[g, pl.ds(EXT + r0 - R * w, R), :]
        o_s[pl.ds(r0 // 2, R // 2), pl.ds(LANES * g, LANES)] = _pack(acc * inv)


def _kernel(x_hbm, wqkv_hbm, wo_hbm, w1_hbm, b1_in, w2_hbm, b2_in, out_hbm,
            wqkv_r, wo_r, wq_s, wk_s, wv_s, wo_s, qh_s, kh_s, w1_s, w2_s, xio_s, xp_s, x1_s, xm_s, xn_s, q_s, k_s, v_s, hk_s, hv_s, o_s,
            b1_ref, b2_ref,
            wsem, xsem, osem, *, T, FC, LAG, ORDER, O_A, O_B, O_C, TFIN, KCH, PRB, TLN, PFREE, DS, DUN, XW):
    S, D = xio_s.shape
    F = w1_s.shape[1]
    NT = S // T
    NC = F // FC
    qscale = (D // H) ** -0.5 * math.log2(math.e)

    RC = D // KCH

    def cp_qkv(p, c):
        r = pl.ds(pl.multiple_of(c * RC, RC), RC)
        cols = pl.ds(pl.multiple_of(p * D, D), D)
        return pltpu.make_async_copy(wqkv_hbm.at[r, cols], wqkv_r.at[p, r], wsem.at[3 + p * KCH + c])

    cp_wo = pltpu.make_async_copy(wo_hbm, wo_r, wsem.at[0])
    cp_w1 = pltpu.make_async_copy(w1_hbm, w1_s, wsem.at[1])
    cp_w2 = pltpu.make_async_copy(w2_hbm, w2_s, wsem.at[2])

    def rows(t):
        return pl.ds(pl.multiple_of(t * T, T), T)

    def cp_x(t):
        return pltpu.make_async_copy(x_hbm.at[rows(t)], xio_s.at[rows(t)], xsem.at[t])

    def cp_out(t):
        return pltpu.make_async_copy(xio_s.at[rows(t)], out_hbm.at[rows(t)], osem.at[t])

    def dot(a, b):
        return jnp.dot(a, b, preferred_element_type=F32)

    def xperm(n):
        xp = _load_rows_permuted(xio_s, pl.multiple_of((n % NT) * T, T), T)
        xp_s[n % (LAG + 1)] = xp
        toks = []
        for hi in range(T // 128):
            for g in range(G):
                t = xp[64 * hi:64 * (hi + 1), LANES * g:LANES * (g + 1)]
                toks.append(pltpu.bitcast(t[0:16] | t[16:32] | t[32:48] | t[48:64], F32))
        return toks

    def tie(x, never, tok):
        if tok is None:
            return x
        x0 = jnp.where(never, tok, x[:, :LANES])
        return x0 if x.shape[1] == LANES else jnp.concatenate([x0, x[:, LANES:]], axis=1)

    def ln1(n, x1, never, toks, a, b):
        out = []
        for i in range(a, b):
            r = pl.ds(8 * i, 8)
            x = tie(_unpack(xp_s[n % (LAG + 1), r, :]).astype(F32), never, toks and toks[i - a])
            y = _layernorm(x)
            x1[r, :] = _pack(y)
            out.append(y[:, D - LANES:])
        return out

    def ln2(n, never, toks, a, b):
        s = n % (LAG + 1)
        out = []
        for i in range(a, b):
            x = tie(xm_s[s, pl.ds(16 * i, 16), :], never, toks and toks[i - a])
            y = _layernorm(x)
            xn_s[s, pl.ds(8 * i, 8), :] = _pack(y)
            out.append(y[:, D - LANES:])
        return out

    def step(na, nf, order, head=False):
        st = {}
        if na is not None:
            ta = na % NT
            sa = na % (LAG + 1)
            never = lax.broadcasted_iota(jnp.int32, (16, LANES), 0) < jnp.minimum(na, 0)
            x1, x1n = (x1_s.at[na], o_s) if head else (x1_s.at[LAG], x1_s.at[LAG])
            qr, kr = (qh_s.at[na], kh_s.at[na]) if head else (q_s, k_s)
        if nf is not None:
            tf = nf % NT
            sf = nf % (LAG + 1)

        def tokens(op, count=T // 16):
            if ":" not in op:
                return None
            cols = []
            op, *pad = op.split("~")
            skip, lead = map(int, pad) if pad else (0, 0)
            for src in op.split(":")[1].split("+"):
                if src not in st:
                    return None
                cols += [(st[src], j) for j in range(st[src].shape[1] // LANES)]
            nb = T // 16
            out = []
            for i in range(count):
                pos = (i + skip) * len(cols) * nb // (count + skip + lead)
                val, j = cols[pos // nb]
                r = 16 * (pos % nb)
                out.append(val[r:r + 16, LANES * j:LANES * (j + 1)])
            return out

        def pull(val, spec):
            if spec is None or spec.split(".")[0] not in st:
                return val
            name, a, b = spec.split(".")
            toks = st[name][int(a):int(b)]
            nc, nb = val.shape[1] // LANES, T // 16
            at = {divmod((2 * i + 1) * nc * nb // (2 * len(toks)), nb): t for i, t in enumerate(toks)}
            cols = []
            for j in range(nc):
                col = val[:, LANES * j:LANES * (j + 1)]
                if any(jj == j for jj, _ in at):
                    col = jnp.concatenate([tie(col[16 * r:16 * (r + 1)], never, at.get((j, r)))
                                           for r in range(nb)], axis=0)
                cols.append(col)
            return jnp.concatenate(cols, axis=1)

        for op in order:
            op, *specs = op.split("/")
            specs = dict(sp.split("<") for sp in specs)
            if op[0] == "f":
                if nf is None:
                    continue
            elif na is None:
                continue
            if op.startswith("ln"):
                a, b = map(int, op.split(":")[0].split("@")[1:] or (0, T // 16))
            if op.startswith("perm"):
                if op.startswith("permq"):
                    h0 = jnp.maximum(na - 1, 0) * (D // 4)
                    jobs = [(_permute_cols_block, wqkv_r.at[jnp.where(na == 0, 1, 0)], wq_s, h0 + 16 * i, 16)
                            for i in range(D // 64)]
                else:
                    nv, no = -(-D // 32 // LAG), -(-G // LAG)
                    h0 = jnp.minimum(na * nv, D // 32 - nv) * 16
                    n0 = jnp.minimum(na * no, G - no)
                    jv = [(_permute_cols_block, wqkv_r.at[2], wv_s, h0 + 16 * i, 16) for i in range(nv)]
                    jo = [(_permute_rows_block, wo_r, wo_s, 32 * (i % 4), n0 + i // 4) for i in range(4 * no)]
                    jobs = [j for pair in zip(jv + [None] * len(jo), jo) for j in pair if j] + jv[len(jo):]
                toks = [None] * PFREE + tokens(op, len(jobs) - PFREE)
                for (fn, *args), tok in zip(jobs, toks):
                    tok = None if tok is None else pltpu.bitcast(tok, U32)
                    fn(*args, hint=functools.partial(tie, never=never, tok=tok))
            elif op == "x1":
                x1[...] = o_s[...]
            elif op == "xp":
                st["xp"] = xperm(na + 1)
            elif op.startswith("ln1"):
                st["l1"] = ln1(na + 1, x1n, never, tokens(op, b - a), a, b)
            elif op == "q":
                st["q"] = pull(dot(_unpack(x1[...]), _unpack(wq_s[...])), specs.get("y"))
                q = st["q"] * qscale
                for g in range(G):
                    qr[g] = q[:, LANES * g:LANES * (g + 1)]
            elif op == "k":
                st["k"] = pull(dot(_unpack(x1[...]), _unpack(wk_s[...])), specs.get("y"))
                _store_kv(st["k"], kr, hk_s, T)
            elif op == "v":
                st["v"] = pull(dot(_unpack(x1[...]), _unpack(wv_s[...])), specs.get("y"))
                _store_kv(st["v"], v_s, hv_s, T)
            elif op == "qk":
                row = lax.broadcasted_iota(jnp.int32, (16, LANES), 0)
                invalid = row < jnp.where(ta == 0, 2, 0)
                st["p"] = [_attn_probs(qr, kr, i, invalid) for i in range(T // 16)]
                st["sm"] = [inv for _, inv in st["p"]]
            elif op == "pv":
                for i in range(T // 16):
                    _attn_values(*st["p"][i], v_s, o_s, i)
            elif op == "wo":
                st["wo"] = _unpack(xp_s[sa]).astype(F32) + pull(dot(_unpack(o_s[...]), _unpack(wo_s[...])), specs.get("y"))
                xm_s[sa] = st["wo"]
            elif op.startswith("ln2"):
                st["l2"] = ln2(na + LAG, never, tokens(op, b - a), a, b)
            elif op == "fbeg":
                st["fxn"] = _unpack(xn_s[sf])
                st["facc"] = xm_s[sf] + b2_ref[...].astype(F32)
            elif op == "fend":
                _store_rows_unpermuted(xio_s, pl.multiple_of(tf * T, T), T, slice(None), st["facc"])
            else:
                c = int(op[1:])
                h = st[f"h{c}"] = pull(dot(st["fxn"], w1_s[:, pl.ds(c * FC, FC)]), specs.get("h"))
                h = _gelu(h + b1_ref[:, pl.ds(c * FC, FC)].astype(F32)).astype(BF16)
                st[f"y{c}"] = pull(dot(h, w2_s[pl.ds(c * FC, FC), :]), specs.get("y"))
                st[f"z{c}"] = st["facc"] = st["facc"] + st[f"y{c}"]

    order = ORDER.split(",")
    assert sorted(int(o[1]) for o in order if o[0] == "f" and o[1].isdigit()) == list(range(NC))

    assert LAG == 3 and KCH == 4
    fetch = ([cp_x(0)] + [cp_qkv(1, c) for c in range(4)] + [cp_x(1), cp_x(2), cp_qkv(0, 0), cp_qkv(0, 1), cp_x(3),
               cp_qkv(0, 2), cp_qkv(0, 3), cp_wo] + [cp_qkv(2, c) for c in range(4)] + [cp_x(4), cp_w1, cp_w2]
               + [cp_x(t) for t in range(5, NT)])
    cuts = (0,) + tuple(DS) + (len(fetch),)

    def issue(stage, when=None):
        cps = fetch[cuts[stage]:cuts[stage + 1]]
        if cps and when is None:
            for cp in cps:
                cp.start()
        elif cps:
            @pl.when(when)
            def _():
                for cp in cps:
                    cp.start()

    issue(0)
    b1_ref[...] = b1_in[...].astype(F32).reshape(1, F)
    b2_ref[...] = b2_in[...].astype(F32).reshape(1, D)
    hk_s[...] = jnp.zeros(hk_s.shape, F32)
    hv_s[...] = jnp.zeros(hv_s.shape, F32)
    cp_x(0).wait()
    issue(1)
    xperm(0)

    def ln_first(i, carry):
        r = pl.ds(pl.multiple_of(i * 32, 32), 32)
        o_s[r, :] = _pack(_layernorm(_unpack(xp_s[0, r, :]).astype(F32)))
        xm_s[LAG, pl.ds(pl.multiple_of(i * 64, 64), 64), :] = jnp.zeros((64, D), F32)
        return carry

    lax.fori_loop(0, T // 64, ln_first, 0)
    issue(2)

    def perm_k(c, carry):
        cp_qkv(1, c).wait()
        issue(3, c == 1)
        issue(4, c == 3)
        for rr in range(0, RC, PRB):
            _permute_cols_block(wqkv_r.at[1], wk_s, c * (RC // 2) + rr // 2, PRB // 2)
        return carry

    lax.fori_loop(0, KCH, perm_k, 0)

    def head_k(n, carry):
        cp_x(n + 1).wait()

        @pl.when(n > 0)
        def _():
            cp_qkv(0, 2 * n - 2).wait()
            cp_qkv(0, 2 * n - 1).wait()

        for i in range(LAG):
            issue(5 + i, n == i)

        step(n, None, O_A.split(","), head=True)
        return carry

    def head_q(n, carry):
        cp_qkv(2, n + 1).wait()
        step(n, None, O_B.split(","), head=True)
        return carry

    def head_v(n, carry):
        step(n, None, O_C.split(","), head=True)
        return carry

    lax.fori_loop(0, LAG, head_k, 0)
    issue(8)
    x1_s[LAG] = o_s[...]
    cp_wo.wait()
    cp_qkv(2, 0).wait()
    lax.fori_loop(0, LAG, head_q, 0)
    lax.fori_loop(0, LAG, head_v, 0)
    cp_w1.wait()
    cp_w2.wait()

    if XW:
        for t in range(LAG + 1, NT):
            cp_x(t).wait()

    def steady(n, carry):
        if not XW:
            @pl.when(n + 1 < NT)
            def _():
                cp_x(n + 1).wait()

        step(n, n - LAG, order)
        return carry

    lax.fori_loop(LAG, 2 * NT, steady, 0)
    for t in range(NT - LAG):
        cp_out(t).start()
    last = 2 * NT - 1
    CW = D // 4

    def finish(n, j, never, toks):
        for g in range(CW // LANES):
            cols = pl.ds(pl.multiple_of(j * CW + g * LANES, LANES), LANES)
            val = xm_s[n % (LAG + 1), :, cols] + b2_ref[:, cols]
            val = jnp.concatenate([tie(val[16 * r:16 * (r + 1)], never, toks.get((g, r))) for r in range(T // 16)], axis=0)
            _store_rows_unpermuted(xio_s, pl.multiple_of((n % NT) * T, T), T, cols, val)

    def tail(n, carry):
        sf = n % (LAG + 1)
        sl = jnp.where(n < last, last, last + 1) % (LAG + 1)

        def chunk(c, carry):
            c0 = pl.multiple_of(c * FC, FC)
            i = jnp.minimum((n - (2 * NT - LAG)) * NC + c, T // 32 - 1)
            x = xm_s[sl, pl.ds(pl.multiple_of(32 * i, 32), 32), :]
            h = dot(_unpack(xn_s[sf]), w1_s[:, pl.ds(c0, FC)])
            if TFIN:
                never = lax.broadcasted_iota(jnp.int32, (16, LANES), 0) < jnp.minimum(n, 0)
                toks = {}
                for u, (tc, tr) in enumerate(TFIN):
                    for r in range(8):
                        toks[(u // 2, 8 * (u % 2) + r)] = h[tr:tr + 16, LANES * tc:LANES * (tc + 1)]
                finish(jnp.maximum(n - 1, 2 * NT - LAG), jnp.minimum(c, 3), never, toks)
            h = _gelu(h + b1_ref[:, pl.ds(c0, FC)]).astype(BF16)
            y = xm_s[sf] + dot(h, w2_s[pl.ds(c0, FC), :])
            xn = _pack(_layernorm(x))
            xn_s[sl, pl.ds(pl.multiple_of(16 * i, 16), 16), :] = xn
            if TLN is not None:
                tok = xn[:, :LANES]
                for g in range(1, G):
                    tok = tok | xn[:, LANES * g:LANES * (g + 1)]
                a = LANES * TLN
                yc = jnp.concatenate([tie(y[:16, a:a + LANES], never, pltpu.bitcast(tok, F32)), y[16:, a:a + LANES]], axis=0)
                y = jnp.concatenate([y[:, :a], yc, y[:, a + LANES:]], axis=1)
            xm_s[sf] = y
            return carry

        lax.fori_loop(0, NC, chunk, 0)
        if TFIN:
            @pl.when(n > 2 * NT - LAG)
            def _():
                cp_out(n - 1 - NT).start()
        else:
            step(None, n, ["fbeg", "fend"])
            cp_out(n - NT).start()
        return carry

    lax.fori_loop(2 * NT - LAG, 2 * NT, tail, 0)

    def cp_last(j):
        cols = pl.ds(pl.multiple_of(j * CW, CW), CW)
        return pltpu.make_async_copy(xio_s.at[rows(NT - 1), cols], out_hbm.at[rows(NT - 1), cols], osem.at[NT - 1 + j])

    def drain(j, carry):
        finish(last, j, None, {})
        cp_last(j).start()
        return carry

    lax.fori_loop(0, D // CW, drain, 0, unroll=DUN)
    for t in range(NT - 1):
        cp_out(t).wait()
    for j in range(D // CW):
        cp_last(j).wait()


def _forward(A_x, A_wqkv, A_wo, B_w1, B_b1, B_w2, B_b2, T=256, FC=512, LAG=3, TFIN=((0,0),(1,0),(2,0),(3,0)), KCH=4, PRB=32, PFREE=1, XW=0, DUN=False, DS=(2, 5, 6, 9, 12, 99, 99, 99), TLN=2,
             ORDER="fbeg,xp,k/y<xp.0.16,q,qk,f0,f1/h<sm.0.8/y<sm.8.16,v,pv,f2,f3,ln2:y2+y3~0~1,f4,f5,ln1:y4+y5~0~1,f6,wo,fend",
             O_A="x1,xp,k,ln1:k~0~2,permq:k~0~2", O_B="q,permv:q~0~2", O_C="qk,v,ln2:v~48~0,pv,wo"):
    B, S, D = A_x.shape
    F = B_w1.shape[1]
    assert B == 1 and D == G * LANES and S % T == 0 and F % FC == 0 and T % 128 == 0 and 2 <= LAG < S // T
    any_spec = pl.BlockSpec(memory_space=pl.ANY)
    vmem_spec = pl.BlockSpec(memory_space=pltpu.VMEM)
    out = pl.pallas_call(
        functools.partial(_kernel, T=T, FC=FC, LAG=LAG, ORDER=ORDER, O_A=O_A, O_B=O_B, O_C=O_C, TFIN=TFIN, KCH=KCH, PRB=PRB, PFREE=PFREE, XW=XW, DUN=DUN, DS=DS, TLN=TLN),
        in_specs=[any_spec, any_spec, any_spec, any_spec, vmem_spec, any_spec, vmem_spec],
        out_specs=any_spec,
        out_shape=jax.ShapeDtypeStruct((S, D), A_x.dtype),
        scratch_shapes=[
            pltpu.VMEM((3, D, D), BF16),
            pltpu.VMEM((D, D), BF16),
            pltpu.VMEM((D // 2, D), U32),
            pltpu.VMEM((D // 2, D), U32),
            pltpu.VMEM((D // 2, D), U32),
            pltpu.VMEM((D // 2, D), U32),
            pltpu.VMEM((LAG, G, T, LANES), F32),
            pltpu.VMEM((LAG, G, T + EXT, LANES), F32),
            pltpu.VMEM((D, F), BF16),
            pltpu.VMEM((F, D), BF16),
            pltpu.VMEM((S, D), BF16),
            pltpu.VMEM((LAG + 1, T // 2, D), U32),
            pltpu.VMEM((LAG + 1, T // 2, D), U32),
            pltpu.VMEM((LAG + 1, T, D), F32),
            pltpu.VMEM((LAG + 1, T // 2, D), U32),
            pltpu.VMEM((G, T, LANES), F32),
            pltpu.VMEM((G, T + EXT, LANES), F32),
            pltpu.VMEM((G, T + EXT, LANES), F32),
            pltpu.VMEM((G, EXT // 2, LANES), F32),
            pltpu.VMEM((G, EXT // 2, LANES), F32),
            pltpu.VMEM((T // 2, D), U32),
            pltpu.VMEM((1, F), F32),
            pltpu.VMEM((1, D), F32),
            pltpu.SemaphoreType.DMA((3 + 3 * KCH,)),
            pltpu.SemaphoreType.DMA((S // T,)),
            pltpu.SemaphoreType.DMA((S // T + 3,)),
        ],
        compiler_params=pltpu.CompilerParams(vmem_limit_bytes=100 * 1024 * 1024),
    )(A_x.reshape(S, D), A_wqkv, A_wo, B_w1, B_b1, B_w2, B_b2)
    return out.reshape(B, S, D)


@jax.jit
def pallas_interleave_layers__sliding_local_dilated__dense_activation_gelu__prompt_kernel(
    A_x: jax.Array,
    A_wqkv: jax.Array,
    A_wo: jax.Array,
    B_x: jax.Array,
    B_w1: jax.Array,
    B_b1: jax.Array,
    B_w2: jax.Array,
    B_b2: jax.Array,
):
    del B_x
    return _forward(A_x, A_wqkv, A_wo, B_w1, B_b1, B_w2, B_b2)
```

```python
import functools
import math

import jax
import jax.numpy as jnp
from jax import lax
import jax.experimental.pallas as pl
import jax.experimental.pallas.tpu as pltpu

H = 32
W = 8
LANES = 128
G = 8
EXT = 16 * (W - 1)
EPS = 1e-5
F32 = jnp.float32
BF16 = jnp.bfloat16
U32 = jnp.uint32


def _layernorm(x):
    m = jnp.mean(x, axis=-1, keepdims=True)
    xc = x - m
    v = jnp.mean(xc * xc, axis=-1, keepdims=True)
    return xc * lax.rsqrt(v + EPS)


def _gelu(x):
    c = math.sqrt(2.0 / math.pi)
    hx = 0.5 * x
    return hx + hx * jnp.tanh(x * (c + (c * 0.044715) * (x * x)))


def _pack(x):
    return pltpu.bitcast(x.astype(BF16), U32)


def _unpack(u):
    return pltpu.bitcast(u, BF16)


def _barrel(tiles, b):
    for t in (1, 2, 4):
        m = (b & t) != 0
        tiles = [jnp.where(m, tiles[(j + t) % 8], tiles[j]) for j in range(8)]
    return tiles


def _permute_cols_block(src_ref, w_ref, h0, hb, hint=lambda t: t):
    rows = pl.ds(pl.multiple_of(2 * h0, 2 * hb), 2 * hb)
    tiles = [_pack(src_ref[rows, pl.ds(LANES * g, LANES)]) for g in range(G)]
    tiles[0] = hint(tiles[0])
    b = (lax.broadcasted_iota(jnp.int32, tiles[0].shape, 1) >> 2) & 7
    tiles = _barrel(tiles, b)
    for j in range(G):
        t = tiles[j]
        if j:
            t = jnp.where(b >= j, pltpu.roll(t, 4 * j, 1), pltpu.roll(t, LANES - 32 + 4 * j, 1))
        w_ref[pl.ds(pl.multiple_of(h0, hb), hb), pl.ds(LANES * j, LANES)] = t


def _permute_rows_block(src_ref, w_ref, r0, n, hint=lambda t: t):
    cols = pl.ds(pl.multiple_of(n * LANES, LANES), LANES)
    tiles = [_pack(src_ref[pl.ds(r0 + LANES * g, 32), cols]) for g in range(G)]
    tiles[0] = hint(tiles[0])
    b = lax.broadcasted_iota(jnp.int32, tiles[0].shape, 0) >> 1
    tiles = _barrel(tiles, b)
    for j in range(G):
        t = pltpu.roll(tiles[j], 2 * j, 0) if j else tiles[j]
        w_ref[pl.ds((r0 + LANES * j) // 2, 16), cols] = t


def _transpose8(tiles):
    sub = lax.broadcasted_iota(jnp.int32, tiles[0].shape, 0)
    for s in (4, 2, 1):
        m = (sub & s) == 0
        new = list(tiles)
        for g in range(8):
            if g & s:
                continue
            x, y = tiles[g], tiles[g | s]
            new[g] = jnp.where(m, x, pltpu.roll(y, s, 0))
            new[g | s] = jnp.where(m, pltpu.roll(x, 8 - s, 0), y)
        tiles = new
    return tiles


def _load_rows_permuted(x_ref, row0, T):
    blocks = []
    for hi in range(T // 128):
        blocks += _transpose8([_pack(x_ref[pl.ds(row0 + u * (T // 8) + 16 * hi, 16), :]) for u in range(8)])
    return jnp.concatenate(blocks, axis=0)


def _store_rows_unpermuted(x_ref, row0, T, cols, val):
    for hi in range(T // 128):
        tiles = _transpose8([_pack(val[128 * hi + 16 * t:128 * hi + 16 * (t + 1), :]) for t in range(8)])
        for u in range(8):
            x_ref[pl.ds(row0 + u * (T // 8) + 16 * hi, 16), cols] = _unpack(tiles[u])


def _store_kv(val, kv_s, halo_s, T):
    first = lax.broadcasted_iota(jnp.int32, (8, LANES), 0) < 2
    for g in range(G):
        col = val[:, LANES * g:LANES * (g + 1)]
        kv_s[g, pl.ds(EXT, T), :] = col
        for e in range(W - 1):
            r = T - EXT + 16 * e
            lo = pltpu.roll(col[r:r + 8], 2, 0)
            hi = pltpu.roll(col[r + 8:r + 16], 2, 0)
            kv_s[g, pl.ds(16 * e, 8), :] = jnp.where(first, halo_s[g, pl.ds(8 * e, 8), :], lo)
            kv_s[g, pl.ds(16 * e + 8, 8), :] = jnp.where(first, lo, hi)
            halo_s[g, pl.ds(8 * e, 8), :] = hi


def _attn_probs(q_s, k_s, i, invalid):
    R = 16
    r0 = R * i
    lane = lax.broadcasted_iota(jnp.int32, (R, LANES), 1)
    m1 = (lane & 1) == 0
    m2 = (lane & 2) == 0
    q = [q_s[g, pl.ds(r0, R), :] for g in range(G)]
    logits = []
    for w in range(W):
        off = EXT + r0 - R * w
        acc = q[0] * k_s[0, pl.ds(off, R), :]
        for g in range(1, G):
            acc = acc + q[g] * k_s[g, pl.ds(off, R), :]
        acc = acc + jnp.where(m1, pltpu.roll(acc, LANES - 1, 1), pltpu.roll(acc, 1, 1))
        acc = acc + jnp.where(m2, pltpu.roll(acc, LANES - 2, 1), pltpu.roll(acc, 2, 1))
        if i < w:
            acc = jnp.where(invalid, -1e9, acc)
        logits.append(acc)
    mx = logits[0]
    for w in range(1, W):
        mx = jnp.maximum(mx, logits[w])
    p = [jnp.exp2(l - mx) for l in logits]
    den = p[0]
    for w in range(1, W):
        den = den + p[w]
    return p, 1.0 / den


def _attn_values(p, inv, v_s, o_s, i):
    R = 16
    r0 = R * i
    for g in range(G):
        acc = p[0] * v_s[g, pl.ds(EXT + r0, R), :]
        for w in range(1, W):
            acc = acc + p[w] * v_s[g, pl.ds(EXT + r0 - R * w, R), :]
        o_s[pl.ds(r0 // 2, R // 2), pl.ds(LANES * g, LANES)] = _pack(acc * inv)


def _kernel(x_hbm, wqkv_hbm, wo_hbm, w1_hbm, b1_in, w2_hbm, b2_in, out_hbm,
            wqkv_r, wo_r, wq_s, wk_s, wv_s, wo_s, qh_s, kh_s, w1_s, w2_s, xio_s, xp_s, x1_s, xm_s, xn_s, q_s, k_s, v_s, hk_s, hv_s, o_s,
            b1_ref, b2_ref,
            wsem, xsem, osem, *, T, FC, LAG, ORDER, O_A, O_B, O_C, TFIN, KCH, PRB, TLN, PFREE, DS, DUN, XW, DC, FT):
    S, D = xio_s.shape
    F = w1_s.shape[1]
    NT = S // T
    NC = F // FC
    qscale = (D // H) ** -0.5 * math.log2(math.e)

    RC = D // KCH

    def cp_qkv(p, c):
        r = pl.ds(pl.multiple_of(c * RC, RC), RC)
        cols = pl.ds(pl.multiple_of(p * D, D), D)
        return pltpu.make_async_copy(wqkv_hbm.at[r, cols], wqkv_r.at[p, r], wsem.at[3 + p * KCH + c])

    cp_wo = pltpu.make_async_copy(wo_hbm, wo_r, wsem.at[0])
    cp_w1 = pltpu.make_async_copy(w1_hbm, w1_s, wsem.at[1])
    cp_w2 = pltpu.make_async_copy(w2_hbm, w2_s, wsem.at[2])

    def rows(t):
        return pl.ds(pl.multiple_of(t * T, T), T)

    def cp_x(t):
        return pltpu.make_async_copy(x_hbm.at[rows(t)], xio_s.at[rows(t)], xsem.at[t])

    def cp_out(t):
        return pltpu.make_async_copy(xio_s.at[rows(t)], out_hbm.at[rows(t)], osem.at[t])

    def dot(a, b):
        return jnp.dot(a, b, preferred_element_type=F32)

    def xperm(n):
        xp = _load_rows_permuted(xio_s, pl.multiple_of((n % NT) * T, T), T)
        xp_s[n % (LAG + 1)] = xp
        toks = []
        for hi in range(T // 128):
            for g in range(G):
                t = xp[64 * hi:64 * (hi + 1), LANES * g:LANES * (g + 1)]
                toks.append(pltpu.bitcast(t[0:16] | t[16:32] | t[32:48] | t[48:64], F32))
        return toks

    def tie(x, never, tok):
        if tok is None:
            return x
        x0 = jnp.where(never, tok, x[:, :LANES])
        return x0 if x.shape[1] == LANES else jnp.concatenate([x0, x[:, LANES:]], axis=1)

    def ln1(n, x1, never, toks, a, b):
        out = []
        for i in range(a, b):
            r = pl.ds(8 * i, 8)
            x = tie(_unpack(xp_s[n % (LAG + 1), r, :]).astype(F32), never, toks and toks[i - a])
            y = _layernorm(x)
            x1[r, :] = _pack(y)
            out.append(y[:, D - LANES:])
        return out

    def ln2(n, never, toks, a, b):
        s = n % (LAG + 1)
        out = []
        for i in range(a, b):
            x = tie(xm_s[s, pl.ds(16 * i, 16), :], never, toks and toks[i - a])
            y = _layernorm(x)
            xn_s[s, pl.ds(8 * i, 8), :] = _pack(y)
            out.append(y[:, D - LANES:])
        return out

    def step(na, nf, order, head=False):
        st = {}
        if na is not None:
            ta = na % NT
            sa = na % (LAG + 1)
            never = lax.broadcasted_iota(jnp.int32, (16, LANES), 0) < jnp.minimum(na, 0)
            x1, x1n = (x1_s.at[na], o_s) if head else (x1_s.at[LAG], x1_s.at[LAG])
            qr, kr = (qh_s.at[na], kh_s.at[na]) if head else (q_s, k_s)
        if nf is not None:
            tf = nf % NT
            sf = nf % (LAG + 1)

        def tokens(op, count=T // 16):
            if ":" not in op:
                return None
            cols = []
            op, *pad = op.split("~")
            skip, lead = map(int, pad) if pad else (0, 0)
            for src in op.split(":")[1].split("+"):
                if src not in st:
                    return None
                cols += [(st[src], j) for j in range(st[src].shape[1] // LANES)]
            nb = T // 16
            out = []
            for i in range(count):
                pos = (i + skip) * len(cols) * nb // (count + skip + lead)
                val, j = cols[pos // nb]
                r = 16 * (pos % nb)
                out.append(val[r:r + 16, LANES * j:LANES * (j + 1)])
            return out

        def pull(val, spec):
            if spec is None or spec.split(".")[0] not in st:
                return val
            name, a, b = spec.split(".")
            toks = st[name][int(a):int(b)]
            nc, nb = val.shape[1] // LANES, T // 16
            at = {divmod((2 * i + 1) * nc * nb // (2 * len(toks)), nb): t for i, t in enumerate(toks)}
            cols = []
            for j in range(nc):
                col = val[:, LANES * j:LANES * (j + 1)]
                if any(jj == j for jj, _ in at):
                    col = jnp.concatenate([tie(col[16 * r:16 * (r + 1)], never, at.get((j, r)))
                                           for r in range(nb)], axis=0)
                cols.append(col)
            return jnp.concatenate(cols, axis=1)

        for op in order:
            op, *specs = op.split("/")
            specs = dict(sp.split("<") for sp in specs)
            if op[0] == "f":
                if nf is None:
                    continue
            elif na is None:
                continue
            if op.startswith("ln"):
                a, b = map(int, op.split(":")[0].split("@")[1:] or (0, T // 16))
            if op.startswith("perm"):
                if op.startswith("permq"):
                    h0 = jnp.maximum(na - 1, 0) * (D // 4)
                    jobs = [(_permute_cols_block, wqkv_r.at[jnp.where(na == 0, 1, 0)], wq_s, h0 + 16 * i, 16)
                            for i in range(D // 64)]
                else:
                    nv, no = -(-D // 32 // LAG), -(-G // LAG)
                    h0 = jnp.minimum(na * nv, D // 32 - nv) * 16
                    n0 = jnp.minimum(na * no, G - no)
                    jv = [(_permute_cols_block, wqkv_r.at[2], wv_s, h0 + 16 * i, 16) for i in range(nv)]
                    jo = [(_permute_rows_block, wo_r, wo_s, 32 * (i % 4), n0 + i // 4) for i in range(4 * no)]
                    jobs = [j for pair in zip(jv + [None] * len(jo), jo) for j in pair if j] + jv[len(jo):]
                toks = [None] * PFREE + tokens(op, len(jobs) - PFREE)
                for (fn, *args), tok in zip(jobs, toks):
                    tok = None if tok is None else pltpu.bitcast(tok, U32)
                    fn(*args, hint=functools.partial(tie, never=never, tok=tok))
            elif op == "x1":
                x1[...] = o_s[...]
            elif op == "xp":
                st["xp"] = xperm(na + 1)
            elif op.startswith("ln1"):
                st["l1"] = ln1(na + 1, x1n, never, tokens(op, b - a), a, b)
            elif op == "q":
                st["q"] = pull(dot(_unpack(x1[...]), _unpack(wq_s[...])), specs.get("y"))
                q = st["q"] * qscale
                for g in range(G):
                    qr[g] = q[:, LANES * g:LANES * (g + 1)]
            elif op == "k":
                st["k"] = pull(dot(_unpack(x1[...]), _unpack(wk_s[...])), specs.get("y"))
                _store_kv(st["k"], kr, hk_s, T)
            elif op == "v":
                st["v"] = pull(dot(_unpack(x1[...]), _unpack(wv_s[...])), specs.get("y"))
                _store_kv(st["v"], v_s, hv_s, T)
            elif op == "qk":
                row = lax.broadcasted_iota(jnp.int32, (16, LANES), 0)
                invalid = row < jnp.where(ta == 0, 2, 0)
                st["p"] = [_attn_probs(qr, kr, i, invalid) for i in range(T // 16)]
                st["sm"] = [inv for _, inv in st["p"]]
            elif op == "pv":
                for i in range(T // 16):
                    _attn_values(*st["p"][i], v_s, o_s, i)
            elif op == "wo":
                st["wo"] = _unpack(xp_s[sa]).astype(F32) + pull(dot(_unpack(o_s[...]), _unpack(wo_s[...])), specs.get("y"))
                xm_s[sa] = st["wo"]
            elif op.startswith("ln2"):
                st["l2"] = ln2(na + LAG, never, tokens(op, b - a), a, b)
            elif op == "fbeg":
                st["fxn"] = _unpack(xn_s[sf])
                st["facc"] = xm_s[sf] + b2_ref[...].astype(F32)
            elif op == "fend":
                _store_rows_unpermuted(xio_s, pl.multiple_of(tf * T, T), T, slice(None), st["facc"])
            else:
                c = int(op[1:])
                h = st[f"h{c}"] = pull(dot(st["fxn"], w1_s[:, pl.ds(c * FC, FC)]), specs.get("h"))
                h = _gelu(h + b1_ref[:, pl.ds(c * FC, FC)].astype(F32)).astype(BF16)
                st[f"y{c}"] = pull(dot(h, w2_s[pl.ds(c * FC, FC), :]), specs.get("y"))
                st[f"z{c}"] = st["facc"] = st["facc"] + st[f"y{c}"]

    order = ORDER.split(",")
    assert sorted(int(o[1]) for o in order if o[0] == "f" and o[1].isdigit()) == list(range(NC))

    assert LAG == 3 and KCH == 4
    fetch = ([cp_x(0)] + [cp_qkv(1, c) for c in range(4)] + [cp_x(1), cp_x(2), cp_qkv(0, 0), cp_qkv(0, 1), cp_x(3),
               cp_qkv(0, 2), cp_qkv(0, 3), cp_wo] + [cp_qkv(2, c) for c in range(4)] + [cp_x(4), cp_w1, cp_w2]
               + [cp_x(t) for t in range(5, NT)])
    cuts = (0,) + tuple(DS) + (len(fetch),)

    def issue(stage, when=None):
        cps = fetch[cuts[stage]:cuts[stage + 1]]
        if cps and when is None:
            for cp in cps:
                cp.start()
        elif cps:
            @pl.when(when)
            def _():
                for cp in cps:
                    cp.start()

    issue(0)
    b1_ref[...] = b1_in[...].astype(F32).reshape(1, F)
    b2_ref[...] = b2_in[...].astype(F32).reshape(1, D)
    hk_s[...] = jnp.zeros(hk_s.shape, F32)
    hv_s[...] = jnp.zeros(hv_s.shape, F32)
    cp_x(0).wait()
    issue(1)
    xperm(0)

    def ln_first(i, carry):
        r = pl.ds(pl.multiple_of(i * 32, 32), 32)
        o_s[r, :] = _pack(_layernorm(_unpack(xp_s[0, r, :]).astype(F32)))
        xm_s[LAG, pl.ds(pl.multiple_of(i * 64, 64), 64), :] = jnp.zeros((64, D), F32)
        return carry

    issue(2)

    def perm_k(c, carry):
        cp_qkv(1, c).wait()
        issue(3, c == DC[0])
        issue(4, c == DC[1])
        ln_first(c, 0)
        for rr in range(0, RC, PRB):
            _permute_cols_block(wqkv_r.at[1], wk_s, c * (RC // 2) + rr // 2, PRB // 2)
        return carry

    lax.fori_loop(0, KCH, perm_k, 0)

    def head_k(n, carry):
        cp_x(n + 1).wait()

        @pl.when(n > 0)
        def _():
            cp_qkv(0, 2 * n - 2).wait()
            cp_qkv(0, 2 * n - 1).wait()

        for i in range(LAG):
            issue(5 + i, n == i)

        step(n, None, O_A.split(","), head=True)
        return carry

    def head_q(n, carry):
        cp_qkv(2, n + 1).wait()
        step(n, None, O_B.split(","), head=True)
        return carry

    def head_v(n, carry):
        step(n, None, O_C.split(","), head=True)
        return carry

    lax.fori_loop(0, LAG, head_k, 0)
    issue(8)
    x1_s[LAG] = o_s[...]
    cp_wo.wait()
    cp_qkv(2, 0).wait()
    lax.fori_loop(0, LAG, head_q, 0)
    lax.fori_loop(0, LAG, head_v, 0)
    cp_w1.wait()
    cp_w2.wait()

    if XW:
        for t in range(LAG + 1, NT):
            cp_x(t).wait()

    def steady(n, carry):
        if not XW:
            @pl.when(n + 1 < NT)
            def _():
                cp_x(n + 1).wait()

        step(n, n - LAG, order)
        return carry

    lax.fori_loop(LAG, 2 * NT, steady, 0)
    for t in range(NT - LAG):
        cp_out(t).start()
    last = 2 * NT - 1
    CW = D // 4

    def finish(n, j, never, toks):
        for g in range(CW // LANES):
            cols = pl.ds(pl.multiple_of(j * CW + g * LANES, LANES), LANES)
            val = xm_s[n % (LAG + 1), :, cols] + b2_ref[:, cols]
            val = jnp.concatenate([tie(val[16 * r:16 * (r + 1)], never, toks.get((g, r))) for r in range(T // 16)], axis=0)
            _store_rows_unpermuted(xio_s, pl.multiple_of((n % NT) * T, T), T, cols, val)

    def tail(n, carry):
        sf = n % (LAG + 1)
        sl = jnp.where(n < last, last, last + 1) % (LAG + 1)

        def chunk(c, carry):
            c0 = pl.multiple_of(c * FT, LANES)
            i = jnp.minimum((n - (2 * NT - LAG)) * (F // FT) + c, T // 32 - 1)
            x = xm_s[sl, pl.ds(pl.multiple_of(32 * i, 32), 32), :]
            h = dot(_unpack(xn_s[sf]), w1_s[:, pl.ds(c0, FT)])
            if TFIN:
                never = lax.broadcasted_iota(jnp.int32, (16, LANES), 0) < jnp.minimum(n, 0)
                toks = {}
                for u, (tc, tr) in enumerate(TFIN):
                    for r in range(8):
                        toks[(u // 2, 8 * (u % 2) + r)] = h[tr:tr + 16, LANES * tc:LANES * (tc + 1)]
                finish(jnp.maximum(n - 1, 2 * NT - LAG), jnp.minimum(c, 3), never, toks)
            h = _gelu(h + b1_ref[:, pl.ds(c0, FT)]).astype(BF16)
            y = xm_s[sf] + dot(h, w2_s[pl.ds(c0, FT), :])
            xn = _pack(_layernorm(x))
            xn_s[sl, pl.ds(pl.multiple_of(16 * i, 16), 16), :] = xn
            if TLN is not None:
                tok = xn[:, :LANES]
                for g in range(1, G):
                    tok = tok | xn[:, LANES * g:LANES * (g + 1)]
                a = LANES * TLN
                yc = jnp.concatenate([tie(y[:16, a:a + LANES], never, pltpu.bitcast(tok, F32)), y[16:, a:a + LANES]], axis=0)
                y = jnp.concatenate([y[:, :a], yc, y[:, a + LANES:]], axis=1)
            xm_s[sf] = y
            return carry

        lax.fori_loop(0, F // FT, chunk, 0)
        if TFIN:
            @pl.when(n > 2 * NT - LAG)
            def _():
                cp_out(n - 1 - NT).start()
        else:
            step(None, n, ["fbeg", "fend"])
            cp_out(n - NT).start()
        return carry

    lax.fori_loop(2 * NT - LAG, 2 * NT, tail, 0)

    def cp_last(j):
        cols = pl.ds(pl.multiple_of(j * CW, CW), CW)
        return pltpu.make_async_copy(xio_s.at[rows(NT - 1), cols], out_hbm.at[rows(NT - 1), cols], osem.at[NT - 1 + j])

    def drain(j, carry):
        finish(last, j, None, {})
        cp_last(j).start()
        return carry

    lax.fori_loop(0, D // CW, drain, 0, unroll=DUN)
    for t in range(NT - 1):
        cp_out(t).wait()
    for j in range(D // CW):
        cp_last(j).wait()


def _forward(A_x, A_wqkv, A_wo, B_w1, B_b1, B_w2, B_b2, T=256, FC=512, LAG=3, TFIN=((0,0),(1,0),(2,0),(3,0)), KCH=4, PRB=32, PFREE=1, FT=896, DC=(1, 3), XW=0, DUN=False, DS=(2, 5, 6, 9, 12, 99, 99, 99), TLN=2,
             ORDER="fbeg,xp,k/y<xp.0.16,q,qk,f0,f1/h<sm.0.8/y<sm.8.16,v,pv,f2,f3,ln2:y2+y3~0~1,f4,f5,ln1:y4+y5~0~1,f6,wo,fend",
             O_A="x1,xp,k,ln1:k~0~2,permq:k~0~2", O_B="q,permv:q~0~2", O_C="qk,v,ln2:v~48~0,pv,wo"):
    B, S, D = A_x.shape
    F = B_w1.shape[1]
    assert B == 1 and D == G * LANES and S % T == 0 and F % FC == 0 and T % 128 == 0 and 2 <= LAG < S // T
    any_spec = pl.BlockSpec(memory_space=pl.ANY)
    vmem_spec = pl.BlockSpec(memory_space=pltpu.VMEM)
    out = pl.pallas_call(
        functools.partial(_kernel, T=T, FC=FC, LAG=LAG, ORDER=ORDER, O_A=O_A, O_B=O_B, O_C=O_C, TFIN=TFIN, KCH=KCH, PRB=PRB, PFREE=PFREE, FT=FT, DC=DC, XW=XW, DUN=DUN, DS=DS, TLN=TLN),
        in_specs=[any_spec, any_spec, any_spec, any_spec, vmem_spec, any_spec, vmem_spec],
        out_specs=any_spec,
        out_shape=jax.ShapeDtypeStruct((S, D), A_x.dtype),
        scratch_shapes=[
            pltpu.VMEM((3, D, D), BF16),
            pltpu.VMEM((D, D), BF16),
            pltpu.VMEM((D // 2, D), U32),
            pltpu.VMEM((D // 2, D), U32),
            pltpu.VMEM((D // 2, D), U32),
            pltpu.VMEM((D // 2, D), U32),
            pltpu.VMEM((LAG, G, T, LANES), F32),
            pltpu.VMEM((LAG, G, T + EXT, LANES), F32),
            pltpu.VMEM((D, F), BF16),
            pltpu.VMEM((F, D), BF16),
            pltpu.VMEM((S, D), BF16),
            pltpu.VMEM((LAG + 1, T // 2, D), U32),
            pltpu.VMEM((LAG + 1, T // 2, D), U32),
            pltpu.VMEM((LAG + 1, T, D), F32),
            pltpu.VMEM((LAG + 1, T // 2, D), U32),
            pltpu.VMEM((G, T, LANES), F32),
            pltpu.VMEM((G, T + EXT, LANES), F32),
            pltpu.VMEM((G, T + EXT, LANES), F32),
            pltpu.VMEM((G, EXT // 2, LANES), F32),
            pltpu.VMEM((G, EXT // 2, LANES), F32),
            pltpu.VMEM((T // 2, D), U32),
            pltpu.VMEM((1, F), F32),
            pltpu.VMEM((1, D), F32),
            pltpu.SemaphoreType.DMA((3 + 3 * KCH,)),
            pltpu.SemaphoreType.DMA((S // T,)),
            pltpu.SemaphoreType.DMA((S // T + 3,)),
        ],
        compiler_params=pltpu.CompilerParams(vmem_limit_bytes=100 * 1024 * 1024),
    )(A_x.reshape(S, D), A_wqkv, A_wo, B_w1, B_b1, B_w2, B_b2)
    return out.reshape(B, S, D)


@jax.jit
def pallas_interleave_layers__sliding_local_dilated__dense_activation_gelu__prompt_kernel(
    A_x: jax.Array,
    A_wqkv: jax.Array,
    A_wo: jax.Array,
    B_x: jax.Array,
    B_w1: jax.Array,
    B_b1: jax.Array,
    B_w2: jax.Array,
    B_b2: jax.Array,
):
    del B_x
    return _forward(A_x, A_wqkv, A_wo, B_w1, B_b1, B_w2, B_b2)
```

```python
import functools
import math

import jax
import jax.numpy as jnp
from jax import lax
import jax.experimental.pallas as pl
import jax.experimental.pallas.tpu as pltpu

H = 32
W = 8
LANES = 128
G = 8
EXT = 16 * (W - 1)
EPS = 1e-5
F32 = jnp.float32
BF16 = jnp.bfloat16
U32 = jnp.uint32


def _layernorm(x):
    m = jnp.mean(x, axis=-1, keepdims=True)
    xc = x - m
    v = jnp.mean(xc * xc, axis=-1, keepdims=True)
    return xc * lax.rsqrt(v + EPS)


def _gelu(x):
    c = math.sqrt(2.0 / math.pi)
    hx = 0.5 * x
    return hx + hx * jnp.tanh(x * (c + (c * 0.044715) * (x * x)))


def _pack(x):
    return pltpu.bitcast(x.astype(BF16), U32)


def _unpack(u):
    return pltpu.bitcast(u, BF16)


def _barrel(tiles, b):
    for t in (1, 2, 4):
        m = (b & t) != 0
        tiles = [jnp.where(m, tiles[(j + t) % 8], tiles[j]) for j in range(8)]
    return tiles


def _permute_cols_block(src_ref, w_ref, h0, hb, hint=lambda t: t):
    rows = pl.ds(pl.multiple_of(2 * h0, 2 * hb), 2 * hb)
    tiles = [_pack(src_ref[rows, pl.ds(LANES * g, LANES)]) for g in range(G)]
    tiles[0] = hint(tiles[0])
    b = (lax.broadcasted_iota(jnp.int32, tiles[0].shape, 1) >> 2) & 7
    tiles = _barrel(tiles, b)
    for j in range(G):
        t = tiles[j]
        if j:
            t = jnp.where(b >= j, pltpu.roll(t, 4 * j, 1), pltpu.roll(t, LANES - 32 + 4 * j, 1))
        w_ref[pl.ds(pl.multiple_of(h0, hb), hb), pl.ds(LANES * j, LANES)] = t


def _permute_rows_block(src_ref, w_ref, r0, n, hint=lambda t: t):
    cols = pl.ds(pl.multiple_of(n * LANES, LANES), LANES)
    tiles = [_pack(src_ref[pl.ds(r0 + LANES * g, 32), cols]) for g in range(G)]
    tiles[0] = hint(tiles[0])
    b = lax.broadcasted_iota(jnp.int32, tiles[0].shape, 0) >> 1
    tiles = _barrel(tiles, b)
    for j in range(G):
        t = pltpu.roll(tiles[j], 2 * j, 0) if j else tiles[j]
        w_ref[pl.ds((r0 + LANES * j) // 2, 16), cols] = t


def _transpose8(tiles):
    sub = lax.broadcasted_iota(jnp.int32, tiles[0].shape, 0)
    for s in (4, 2, 1):
        m = (sub & s) == 0
        new = list(tiles)
        for g in range(8):
            if g & s:
                continue
            x, y = tiles[g], tiles[g | s]
            new[g] = jnp.where(m, x, pltpu.roll(y, s, 0))
            new[g | s] = jnp.where(m, pltpu.roll(x, 8 - s, 0), y)
        tiles = new
    return tiles


def _load_rows_permuted(x_ref, row0, T):
    blocks = []
    for hi in range(T // 128):
        blocks += _transpose8([_pack(x_ref[pl.ds(row0 + u * (T // 8) + 16 * hi, 16), :]) for u in range(8)])
    return jnp.concatenate(blocks, axis=0)


def _store_rows_unpermuted(x_ref, row0, T, cols, val):
    for hi in range(T // 128):
        tiles = _transpose8([_pack(val[128 * hi + 16 * t:128 * hi + 16 * (t + 1), :]) for t in range(8)])
        for u in range(8):
            x_ref[pl.ds(row0 + u * (T // 8) + 16 * hi, 16), cols] = _unpack(tiles[u])


def _store_kv(val, kv_s, halo_s, T):
    first = lax.broadcasted_iota(jnp.int32, (8, LANES), 0) < 2
    for g in range(G):
        col = val[:, LANES * g:LANES * (g + 1)]
        kv_s[g, pl.ds(EXT, T), :] = col
        for e in range(W - 1):
            r = T - EXT + 16 * e
            lo = pltpu.roll(col[r:r + 8], 2, 0)
            hi = pltpu.roll(col[r + 8:r + 16], 2, 0)
            kv_s[g, pl.ds(16 * e, 8), :] = jnp.where(first, halo_s[g, pl.ds(8 * e, 8), :], lo)
            kv_s[g, pl.ds(16 * e + 8, 8), :] = jnp.where(first, lo, hi)
            halo_s[g, pl.ds(8 * e, 8), :] = hi


def _attn_probs(q_s, k_s, i, invalid):
    R = 16
    r0 = R * i
    lane = lax.broadcasted_iota(jnp.int32, (R, LANES), 1)
    m1 = (lane & 1) == 0
    m2 = (lane & 2) == 0
    q = [q_s[g, pl.ds(r0, R), :] for g in range(G)]
    logits = []
    for w in range(W):
        off = EXT + r0 - R * w
        acc = q[0] * k_s[0, pl.ds(off, R), :]
        for g in range(1, G):
            acc = acc + q[g] * k_s[g, pl.ds(off, R), :]
        acc = acc + jnp.where(m1, pltpu.roll(acc, LANES - 1, 1), pltpu.roll(acc, 1, 1))
        acc = acc + jnp.where(m2, pltpu.roll(acc, LANES - 2, 1), pltpu.roll(acc, 2, 1))
        if i < w:
            acc = jnp.where(invalid, -1e9, acc)
        logits.append(acc)
    mx = logits[0]
    for w in range(1, W):
        mx = jnp.maximum(mx, logits[w])
    p = [jnp.exp2(l - mx) for l in logits]
    den = p[0]
    for w in range(1, W):
        den = den + p[w]
    return p, 1.0 / den


def _attn_values(p, inv, v_s, o_s, i):
    R = 16
    r0 = R * i
    for g in range(G):
        acc = p[0] * v_s[g, pl.ds(EXT + r0, R), :]
        for w in range(1, W):
            acc = acc + p[w] * v_s[g, pl.ds(EXT + r0 - R * w, R), :]
        o_s[pl.ds(r0 // 2, R // 2), pl.ds(LANES * g, LANES)] = _pack(acc * inv)


def _kernel(x_hbm, wqkv_hbm, wo_hbm, w1_hbm, b1_in, w2_hbm, b2_in, out_hbm,
            wqkv_r, wo_r, wq_s, wk_s, wv_s, wo_s, qh_s, kh_s, w1_s, w2_s, xio_s, xp_s, x1_s, xm_s, xn_s, q_s, k_s, v_s, hk_s, hv_s, o_s,
            b1_ref, b2_ref,
            wsem, xsem, osem, *, T, FC, LAG, ORDER, O_A, O_B, O_C, TFIN, KCH, PRB, TLN, PFREE, DS, DC, FT):
    S, D = xio_s.shape
    F = w1_s.shape[1]
    NT = S // T
    NC = F // FC
    qscale = (D // H) ** -0.5 * math.log2(math.e)

    RC = D // KCH

    def cp_qkv(p, c):
        r = pl.ds(pl.multiple_of(c * RC, RC), RC)
        cols = pl.ds(pl.multiple_of(p * D, D), D)
        return pltpu.make_async_copy(wqkv_hbm.at[r, cols], wqkv_r.at[p, r], wsem.at[3 + p * KCH + c])

    cp_wo = pltpu.make_async_copy(wo_hbm, wo_r, wsem.at[0])
    cp_w1 = pltpu.make_async_copy(w1_hbm, w1_s, wsem.at[1])
    cp_w2 = pltpu.make_async_copy(w2_hbm, w2_s, wsem.at[2])

    def rows(t):
        return pl.ds(pl.multiple_of(t * T, T), T)

    def cp_x(t):
        return pltpu.make_async_copy(x_hbm.at[rows(t)], xio_s.at[rows(t)], xsem.at[t])

    def cp_out(t):
        return pltpu.make_async_copy(xio_s.at[rows(t)], out_hbm.at[rows(t)], osem.at[t])

    def dot(a, b):
        return jnp.dot(a, b, preferred_element_type=F32)

    def xperm(n):
        xp = _load_rows_permuted(xio_s, pl.multiple_of((n % NT) * T, T), T)
        xp_s[n % (LAG + 1)] = xp
        toks = []
        for hi in range(T // 128):
            for g in range(G):
                t = xp[64 * hi:64 * (hi + 1), LANES * g:LANES * (g + 1)]
                toks.append(pltpu.bitcast(t[0:16] | t[16:32] | t[32:48] | t[48:64], F32))
        return toks

    def tie(x, never, tok):
        if tok is None:
            return x
        x0 = jnp.where(never, tok, x[:, :LANES])
        return x0 if x.shape[1] == LANES else jnp.concatenate([x0, x[:, LANES:]], axis=1)

    def ln1(n, x1, never, toks, a, b):
        out = []
        for i in range(a, b):
            r = pl.ds(8 * i, 8)
            x = tie(_unpack(xp_s[n % (LAG + 1), r, :]).astype(F32), never, toks and toks[i - a])
            y = _layernorm(x)
            x1[r, :] = _pack(y)
            out.append(y[:, D - LANES:])
        return out

    def ln2(n, never, toks, a, b):
        s = n % (LAG + 1)
        out = []
        for i in range(a, b):
            x = tie(xm_s[s, pl.ds(16 * i, 16), :], never, toks and toks[i - a])
            y = _layernorm(x)
            xn_s[s, pl.ds(8 * i, 8), :] = _pack(y)
            out.append(y[:, D - LANES:])
        return out

    def step(na, nf, order, head=False):
        st = {}
        if na is not None:
            ta = na % NT
            sa = na % (LAG + 1)
            never = lax.broadcasted_iota(jnp.int32, (16, LANES), 0) < jnp.minimum(na, 0)
            x1, x1n = (x1_s.at[na], o_s) if head else (x1_s.at[LAG], x1_s.at[LAG])
            qr, kr = (qh_s.at[na], kh_s.at[na]) if head else (q_s, k_s)
        if nf is not None:
            tf = nf % NT
            sf = nf % (LAG + 1)

        def tokens(op, count=T // 16):
            if ":" not in op:
                return None
            cols = []
            op, *pad = op.split("~")
            skip, lead = map(int, pad) if pad else (0, 0)
            for src in op.split(":")[1].split("+"):
                if src not in st:
                    return None
                cols += [(st[src], j) for j in range(st[src].shape[1] // LANES)]
            nb = T // 16
            out = []
            for i in range(count):
                pos = (i + skip) * len(cols) * nb // (count + skip + lead)
                val, j = cols[pos // nb]
                r = 16 * (pos % nb)
                out.append(val[r:r + 16, LANES * j:LANES * (j + 1)])
            return out

        def pull(val, spec):
            if spec is None or spec.split(".")[0] not in st:
                return val
            name, a, b = spec.split(".")
            toks = st[name][int(a):int(b)]
            nc, nb = val.shape[1] // LANES, T // 16
            at = {divmod((2 * i + 1) * nc * nb // (2 * len(toks)), nb): t for i, t in enumerate(toks)}
            cols = []
            for j in range(nc):
                col = val[:, LANES * j:LANES * (j + 1)]
                if any(jj == j for jj, _ in at):
                    col = jnp.concatenate([tie(col[16 * r:16 * (r + 1)], never, at.get((j, r)))
                                           for r in range(nb)], axis=0)
                cols.append(col)
            return jnp.concatenate(cols, axis=1)

        for op in order:
            op, *specs = op.split("/")
            specs = dict(sp.split("<") for sp in specs)
            if op[0] == "f":
                if nf is None:
                    continue
            elif na is None:
                continue
            if op.startswith("ln"):
                a, b = map(int, op.split(":")[0].split("@")[1:] or (0, T // 16))
            if op.startswith("perm"):
                if op.startswith("permq"):
                    h0 = jnp.maximum(na - 1, 0) * (D // 4)
                    jobs = [(_permute_cols_block, wqkv_r.at[jnp.where(na == 0, 1, 0)], wq_s, h0 + 16 * i, 16)
                            for i in range(D // 64)]
                else:
                    nv, no = -(-D // 32 // LAG), -(-G // LAG)
                    h0 = jnp.minimum(na * nv, D // 32 - nv) * 16
                    n0 = jnp.minimum(na * no, G - no)
                    jv = [(_permute_cols_block, wqkv_r.at[2], wv_s, h0 + 16 * i, 16) for i in range(nv)]
                    jo = [(_permute_rows_block, wo_r, wo_s, 32 * (i % 4), n0 + i // 4) for i in range(4 * no)]
                    jobs = [j for pair in zip(jv + [None] * len(jo), jo) for j in pair if j] + jv[len(jo):]
                toks = [None] * PFREE + tokens(op, len(jobs) - PFREE)
                for (fn, *args), tok in zip(jobs, toks):
                    tok = None if tok is None else pltpu.bitcast(tok, U32)
                    fn(*args, hint=functools.partial(tie, never=never, tok=tok))
            elif op == "x1":
                x1[...] = o_s[...]
            elif op == "xp":
                st["xp"] = xperm(na + 1)
            elif op.startswith("ln1"):
                st["l1"] = ln1(na + 1, x1n, never, tokens(op, b - a), a, b)
            elif op == "q":
                st["q"] = pull(dot(_unpack(x1[...]), _unpack(wq_s[...])), specs.get("y"))
                q = st["q"] * qscale
                for g in range(G):
                    qr[g] = q[:, LANES * g:LANES * (g + 1)]
            elif op == "k":
                st["k"] = pull(dot(_unpack(x1[...]), _unpack(wk_s[...])), specs.get("y"))
                _store_kv(st["k"], kr, hk_s, T)
            elif op == "v":
                st["v"] = pull(dot(_unpack(x1[...]), _unpack(wv_s[...])), specs.get("y"))
                _store_kv(st["v"], v_s, hv_s, T)
            elif op == "qk":
                row = lax.broadcasted_iota(jnp.int32, (16, LANES), 0)
                invalid = row < jnp.where(ta == 0, 2, 0)
                st["p"] = [_attn_probs(qr, kr, i, invalid) for i in range(T // 16)]
                st["sm"] = [inv for _, inv in st["p"]]
            elif op == "pv":
                for i in range(T // 16):
                    _attn_values(*st["p"][i], v_s, o_s, i)
            elif op == "wo":
                st["wo"] = _unpack(xp_s[sa]).astype(F32) + pull(dot(_unpack(o_s[...]), _unpack(wo_s[...])), specs.get("y"))
                xm_s[sa] = st["wo"]
            elif op.startswith("ln2"):
                st["l2"] = ln2(na + LAG, never, tokens(op, b - a), a, b)
            elif op == "fbeg":
                st["fxn"] = _unpack(xn_s[sf])
                st["facc"] = xm_s[sf] + b2_ref[...].astype(F32)
            elif op == "fend":
                _store_rows_unpermuted(xio_s, pl.multiple_of(tf * T, T), T, slice(None), st["facc"])
            else:
                c = int(op[1:])
                h = st[f"h{c}"] = pull(dot(st["fxn"], w1_s[:, pl.ds(c * FC, FC)]), specs.get("h"))
                h = _gelu(h + b1_ref[:, pl.ds(c * FC, FC)].astype(F32)).astype(BF16)
                st[f"y{c}"] = pull(dot(h, w2_s[pl.ds(c * FC, FC), :]), specs.get("y"))
                st[f"z{c}"] = st["facc"] = st["facc"] + st[f"y{c}"]

    order = ORDER.split(",")
    assert sorted(int(o[1]) for o in order if o[0] == "f" and o[1].isdigit()) == list(range(NC))

    assert LAG == 3 and KCH == 4 and T == 64 * KCH and F % FT == 0 and F // FT >= 4
    fetch = ([cp_x(0)] + [cp_qkv(1, c) for c in range(4)] + [cp_x(1), cp_x(2), cp_qkv(0, 0), cp_qkv(0, 1), cp_x(3),
               cp_qkv(0, 2), cp_qkv(0, 3), cp_wo] + [cp_qkv(2, c) for c in range(4)] + [cp_x(4), cp_w1, cp_w2]
               + [cp_x(t) for t in range(5, NT)])
    cuts = (0,) + tuple(DS) + (len(fetch),)

    def issue(stage, when=None):
        cps = fetch[cuts[stage]:cuts[stage + 1]]
        if cps and when is None:
            for cp in cps:
                cp.start()
        elif cps:
            @pl.when(when)
            def _():
                for cp in cps:
                    cp.start()

    issue(0)
    b1_ref[...] = b1_in[...].astype(F32).reshape(1, F)
    b2_ref[...] = b2_in[...].astype(F32).reshape(1, D)
    hk_s[...] = jnp.zeros(hk_s.shape, F32)
    hv_s[...] = jnp.zeros(hv_s.shape, F32)
    cp_x(0).wait()
    issue(1)
    xperm(0)

    def ln_first(i, carry):
        r = pl.ds(pl.multiple_of(i * 32, 32), 32)
        o_s[r, :] = _pack(_layernorm(_unpack(xp_s[0, r, :]).astype(F32)))
        xm_s[LAG, pl.ds(pl.multiple_of(i * 64, 64), 64), :] = jnp.zeros((64, D), F32)
        return carry

    issue(2)

    def perm_k(c, carry):
        cp_qkv(1, c).wait()
        issue(3, c == DC[0])
        issue(4, c == DC[1])
        ln_first(c, 0)
        for rr in range(0, RC, PRB):
            _permute_cols_block(wqkv_r.at[1], wk_s, c * (RC // 2) + rr // 2, PRB // 2)
        return carry

    lax.fori_loop(0, KCH, perm_k, 0)

    def head_k(n, carry):
        cp_x(n + 1).wait()

        @pl.when(n > 0)
        def _():
            cp_qkv(0, 2 * n - 2).wait()
            cp_qkv(0, 2 * n - 1).wait()

        for i in range(LAG):
            issue(5 + i, n == i)

        step(n, None, O_A.split(","), head=True)
        return carry

    def head_q(n, carry):
        cp_qkv(2, n + 1).wait()
        step(n, None, O_B.split(","), head=True)
        return carry

    def head_v(n, carry):
        step(n, None, O_C.split(","), head=True)
        return carry

    lax.fori_loop(0, LAG, head_k, 0)
    issue(8)
    x1_s[LAG] = o_s[...]
    cp_wo.wait()
    cp_qkv(2, 0).wait()
    lax.fori_loop(0, LAG, head_q, 0)
    lax.fori_loop(0, LAG, head_v, 0)
    cp_w1.wait()
    cp_w2.wait()

    def steady(n, carry):
        @pl.when(n + 1 < NT)
        def _():
            cp_x(n + 1).wait()

        step(n, n - LAG, order)
        return carry

    lax.fori_loop(LAG, 2 * NT, steady, 0)
    for t in range(NT - LAG):
        cp_out(t).start()

    last = 2 * NT - 1
    CW = D // 4

    def finish(n, j, never, toks):
        for g in range(CW // LANES):
            cols = pl.ds(pl.multiple_of(j * CW + g * LANES, LANES), LANES)
            val = xm_s[n % (LAG + 1), :, cols] + b2_ref[:, cols]
            val = jnp.concatenate([tie(val[16 * r:16 * (r + 1)], never, toks.get((g, r))) for r in range(T // 16)], axis=0)
            _store_rows_unpermuted(xio_s, pl.multiple_of((n % NT) * T, T), T, cols, val)

    def tail(n, carry):
        sf = n % (LAG + 1)
        sl = jnp.where(n < last, last, last + 1) % (LAG + 1)

        def chunk(c, carry):
            c0 = pl.multiple_of(c * FT, LANES)
            i = jnp.minimum((n - (2 * NT - LAG)) * (F // FT) + c, T // 32 - 1)
            x = xm_s[sl, pl.ds(pl.multiple_of(32 * i, 32), 32), :]
            h = dot(_unpack(xn_s[sf]), w1_s[:, pl.ds(c0, FT)])
            never = lax.broadcasted_iota(jnp.int32, (16, LANES), 0) < jnp.minimum(n, 0)
            toks = {}
            for u, (tc, tr) in enumerate(TFIN):
                for r in range(8):
                    toks[(u // 2, 8 * (u % 2) + r)] = h[tr:tr + 16, LANES * tc:LANES * (tc + 1)]
            finish(jnp.maximum(n - 1, 2 * NT - LAG), jnp.minimum(c, 3), never, toks)
            h = _gelu(h + b1_ref[:, pl.ds(c0, FT)]).astype(BF16)
            y = xm_s[sf] + dot(h, w2_s[pl.ds(c0, FT), :])
            xn = _pack(_layernorm(x))
            xn_s[sl, pl.ds(pl.multiple_of(16 * i, 16), 16), :] = xn
            tok = xn[:, :LANES]
            for g in range(1, G):
                tok = tok | xn[:, LANES * g:LANES * (g + 1)]
            a = LANES * TLN
            yc = jnp.concatenate([tie(y[:16, a:a + LANES], never, pltpu.bitcast(tok, F32)), y[16:, a:a + LANES]], axis=0)
            y = jnp.concatenate([y[:, :a], yc, y[:, a + LANES:]], axis=1)
            xm_s[sf] = y
            return carry

        lax.fori_loop(0, F // FT, chunk, 0)

        @pl.when(n > 2 * NT - LAG)
        def _():
            cp_out(n - 1 - NT).start()

        return carry

    lax.fori_loop(2 * NT - LAG, 2 * NT, tail, 0)

    def cp_last(j):
        cols = pl.ds(pl.multiple_of(j * CW, CW), CW)
        return pltpu.make_async_copy(xio_s.at[rows(NT - 1), cols], out_hbm.at[rows(NT - 1), cols], osem.at[NT - 1 + j])

    def drain(j, carry):
        finish(last, j, None, {})
        cp_last(j).start()
        return carry

    lax.fori_loop(0, D // CW, drain, 0)
    for t in range(NT - 1):
        cp_out(t).wait()
    for j in range(D // CW):
        cp_last(j).wait()


def _forward(A_x, A_wqkv, A_wo, B_w1, B_b1, B_w2, B_b2, T=256, FC=512, LAG=3, TFIN=((0,0),(1,0),(2,0),(3,0)), KCH=4, PRB=32, PFREE=1, FT=896, DC=(1, 3), DS=(2, 5, 7, 9, 12, 17, 99, 99), TLN=1,
             ORDER="fbeg,xp,k/y<xp.0.16,q,qk,f0,f1/h<sm.0.8/y<sm.8.16,v,pv,f2,f3,ln2:y2+y3~0~1,f4,f5,ln1:y4+y5~0~1,f6,wo,fend",
             O_A="x1,xp,k,ln1:k~0~2,permq:k~0~2", O_B="q,permv:q~0~2", O_C="qk,v,ln2:v~48~0,pv,wo"):
    B, S, D = A_x.shape
    F = B_w1.shape[1]
    assert B == 1 and D == G * LANES and S % T == 0 and F % FC == 0 and T % 128 == 0 and 2 <= LAG < S // T
    any_spec = pl.BlockSpec(memory_space=pl.ANY)
    vmem_spec = pl.BlockSpec(memory_space=pltpu.VMEM)
    out = pl.pallas_call(
        functools.partial(_kernel, T=T, FC=FC, LAG=LAG, ORDER=ORDER, O_A=O_A, O_B=O_B, O_C=O_C, TFIN=TFIN, KCH=KCH, PRB=PRB, PFREE=PFREE, FT=FT, DC=DC, DS=DS, TLN=TLN),
        in_specs=[any_spec, any_spec, any_spec, any_spec, vmem_spec, any_spec, vmem_spec],
        out_specs=any_spec,
        out_shape=jax.ShapeDtypeStruct((S, D), A_x.dtype),
        scratch_shapes=[
            pltpu.VMEM((3, D, D), BF16),
            pltpu.VMEM((D, D), BF16),
            pltpu.VMEM((D // 2, D), U32),
            pltpu.VMEM((D // 2, D), U32),
            pltpu.VMEM((D // 2, D), U32),
            pltpu.VMEM((D // 2, D), U32),
            pltpu.VMEM((LAG, G, T, LANES), F32),
            pltpu.VMEM((LAG, G, T + EXT, LANES), F32),
            pltpu.VMEM((D, F), BF16),
            pltpu.VMEM((F, D), BF16),
            pltpu.VMEM((S, D), BF16),
            pltpu.VMEM((LAG + 1, T // 2, D), U32),
            pltpu.VMEM((LAG + 1, T // 2, D), U32),
            pltpu.VMEM((LAG + 1, T, D), F32),
            pltpu.VMEM((LAG + 1, T // 2, D), U32),
            pltpu.VMEM((G, T, LANES), F32),
            pltpu.VMEM((G, T + EXT, LANES), F32),
            pltpu.VMEM((G, T + EXT, LANES), F32),
            pltpu.VMEM((G, EXT // 2, LANES), F32),
            pltpu.VMEM((G, EXT // 2, LANES), F32),
            pltpu.VMEM((T // 2, D), U32),
            pltpu.VMEM((1, F), F32),
            pltpu.VMEM((1, D), F32),
            pltpu.SemaphoreType.DMA((3 + 3 * KCH,)),
            pltpu.SemaphoreType.DMA((S // T,)),
            pltpu.SemaphoreType.DMA((S // T + 3,)),
        ],
        compiler_params=pltpu.CompilerParams(vmem_limit_bytes=100 * 1024 * 1024),
    )(A_x.reshape(S, D), A_wqkv, A_wo, B_w1, B_b1, B_w2, B_b2)
    return out.reshape(B, S, D)


@jax.jit
def pallas_interleave_layers__sliding_local_dilated__dense_activation_gelu__prompt_kernel(
    A_x: jax.Array,
    A_wqkv: jax.Array,
    A_wo: jax.Array,
    B_x: jax.Array,
    B_w1: jax.Array,
    B_b1: jax.Array,
    B_w2: jax.Array,
    B_b2: jax.Array,
):
    del B_x
    return _forward(A_x, A_wqkv, A_wo, B_w1, B_b1, B_w2, B_b2)
```
